```python
import os as _os
_os.environ.setdefault("JAX_PLATFORMS", "cpu")
import jax
import jax.numpy as jnp

def _softmax(x, axis=-1):
    return jax.nn.softmax(x, axis=axis)
def _gelu(x):
    return jax.nn.gelu(x, approximate=True)
def _silu(x):
    return jax.nn.silu(x)
def _sigmoid(x):
    return jax.nn.sigmoid(x)
def _layernorm(x, axis=-1, eps=1e-5):
    m = jnp.mean(x, axis=axis, keepdims=True)
    v = jnp.var(x, axis=axis, keepdims=True)
    return (x - m) / jnp.sqrt(v + eps)
def _scatter_add(tgt, idx, src, axis=0):
    return tgt.at[idx].add(src)
def _segment_sum(src, seg, n):
    return jax.ops.segment_sum(src, seg, n)
class _Rng:
    def __init__(self, key):
        self._k = key
    def _next(self):
        self._k, sub = jax.random.split(self._k)
        return sub
    def normal(self, shape):
        return jax.random.normal(self._next(), shape, dtype=jnp.bfloat16)
    def randint(self, lo, hi, shape):
        return jax.random.randint(self._next(), shape, lo, hi, dtype=jnp.int32)
    def uniform(self, shape, lo=0.0, hi=1.0):
        return jax.random.uniform(self._next(), shape, jnp.bfloat16, lo, hi)
    def permutation(self, n):
        return jax.random.permutation(self._next(), n)


kernel_name = 'gated_mix__ssm_conv_h3__ssm_conv_h3__prompt'

def setup_inputs():
    _rng = _Rng(jax.random.key(int.from_bytes(__import__("os").urandom(4), "little")))
    _w = (lambda a: (lambda t: t.astype(jnp.bfloat16) if jnp.issubdtype(t.dtype, jnp.floating) else t)(jnp.asarray(a)))
    def _A_setup():
        B, S, D = 1, 2048, 640
        ks = 4
        return {
            "q": _w((lambda *s: _rng.normal(s) * 0.05)(B, S, D)),
            "k": _w((lambda *s: _rng.normal(s) * 0.05)(B, S, D)),
            "v": _w((lambda *s: _rng.normal(s) * 0.05)(B, S, D)),
            "shift_k": _w((lambda *s: _rng.normal(s) * 0.05)(D, ks) * 0.5),
            "ssm_k": _w((lambda *s: _rng.normal(s) * 0.05)(D, S) * (1.0 / S ** 0.5)),
            "ssm_D": _w((lambda *s: _rng.normal(s) * 0.05)(D)),
        }
    _A_in = _A_setup()

    def _B_setup():
        B, S, D = 1, 2048, 640
        ks = 4
        return {
            "q": _w((lambda *s: _rng.normal(s) * 0.05)(B, S, D)),
            "k": _w((lambda *s: _rng.normal(s) * 0.05)(B, S, D)),
            "v": _w((lambda *s: _rng.normal(s) * 0.05)(B, S, D)),
            "shift_k": _w((lambda *s: _rng.normal(s) * 0.05)(D, ks) * 0.5),
            "ssm_k": _w((lambda *s: _rng.normal(s) * 0.05)(D, S) * (1.0 / S ** 0.5)),
            "ssm_D": _w((lambda *s: _rng.normal(s) * 0.05)(D)),
        }
    _B_in = _B_setup()

    return {
        "A_q": _A_in["q"],
        "A_k": _A_in["k"],
        "A_v": _A_in["v"],
        "A_shift_k": _A_in["shift_k"],
        "A_ssm_k": _A_in["ssm_k"],
        "A_ssm_D": _A_in["ssm_D"],
        "B_q": _B_in["q"],
        "B_k": _B_in["k"],
        "B_v": _B_in["v"],
        "B_shift_k": _B_in["shift_k"],
        "B_ssm_k": _B_in["ssm_k"],
        "B_ssm_D": _B_in["ssm_D"],
        "gate_w": _w((lambda *s: _rng.normal(s) * 0.05)(640) * 16.0),
    }

def reference(A_q, A_k, A_v, A_shift_k, A_ssm_k, A_ssm_D, B_q, B_k, B_v, B_shift_k, B_ssm_k, B_ssm_D, gate_w):
    def _A_ref(q, k, v, shift_k, ssm_k, ssm_D):
        B, S, D = q.shape
        ks = shift_k.shape[-1]
        k_pad = jnp.pad(k, ((0, 0), (ks - 1, 0), (0, 0)))
        k_shift = jnp.zeros_like(k)
        for t in range(ks):
            k_shift = k_shift + k_pad[:, t:t + S, :] * shift_k[:, ks - 1 - t][None, None, :]
        kv = k_shift * v
        L = 2 * S
        kv_pad = jnp.pad(kv, ((0, 0), (0, S), (0, 0)))
        kf_pad = jnp.pad(ssm_k, ((0, 0), (0, S)))
        kv_f = (lambda x, axes=(-2,-1): jnp.fft.rfft2(x.astype(jnp.float32), axes=axes))(kv_pad[:, None, :, :], axes=(1, 2))
        kf_f = (lambda x, axes=(-2,-1): jnp.fft.rfft2(x.astype(jnp.float32), axes=axes))(kf_pad[:, None, :], axes=(1, 2))
        kf_f = (lambda x, *d: x.transpose(*d))(kf_f, 1, 2, 0)
        y_f = kv_f * kf_f[None, :, :, :]
        y = (lambda x, s, axes=(-2,-1): jnp.fft.irfft2(x, s=s, axes=axes).astype(jnp.bfloat16))(y_f, (1, L), axes=(1, 2))[:, 0, :S, :]
        y = y + kv * ssm_D[None, None, :]
        return q * y

    def _B_ref(q, k, v, shift_k, ssm_k, ssm_D):
        B, S, D = q.shape
        ks = shift_k.shape[-1]
        k_pad = jnp.pad(k, ((0, 0), (ks - 1, 0), (0, 0)))
        k_shift = jnp.zeros_like(k)
        for t in range(ks):
            k_shift = k_shift + k_pad[:, t:t + S, :] * shift_k[:, ks - 1 - t][None, None, :]
        kv = k_shift * v
        L = 2 * S
        kv_pad = jnp.pad(kv, ((0, 0), (0, S), (0, 0)))
        kf_pad = jnp.pad(ssm_k, ((0, 0), (0, S)))
        kv_f = (lambda x, axes=(-2,-1): jnp.fft.rfft2(x.astype(jnp.float32), axes=axes))(kv_pad[:, None, :, :], axes=(1, 2))
        kf_f = (lambda x, axes=(-2,-1): jnp.fft.rfft2(x.astype(jnp.float32), axes=axes))(kf_pad[:, None, :], axes=(1, 2))
        kf_f = (lambda x, *d: x.transpose(*d))(kf_f, 1, 2, 0)
        y_f = kv_f * kf_f[None, :, :, :]
        y = (lambda x, s, axes=(-2,-1): jnp.fft.irfft2(x, s=s, axes=axes).astype(jnp.bfloat16))(y_f, (1, L), axes=(1, 2))[:, 0, :S, :]
        y = y + kv * ssm_D[None, None, :]
        return q * y

    x = A_q
    g = _sigmoid((x * gate_w).sum(-1, keepdims=True))
    a = _A_ref(x, A_k, A_v, A_shift_k, A_ssm_k, A_ssm_D)
    b = _B_ref(x, B_k, B_v, B_shift_k, B_ssm_k, B_ssm_D)
    return g * a + (1 - g) * b
```

```python
import numpy as np
import jax
import jax.numpy as jnp
import jax.experimental.pallas as pl
import jax.experimental.pallas.tpu as pltpu
import ml_dtypes

S = 2048
D = 640
NG = 5
M = 1024
F32 = jnp.float32
BF16 = jnp.bfloat16
EF = 1
FD = 1
ID = 0
ED = 0
SPLIT = 0
LEAD = 4
BC = 0
EXP = []
NOWHEN = 0
NOSCOPE = 0
SPL = [1]
GP = 0
GM = 1


def _pack_rows(x):
    b = np.ascontiguousarray(x).astype(ml_dtypes.bfloat16).view(np.uint16).astype(np.uint32)
    return b[..., 0::2, :] | (b[..., 1::2, :] << 16)


def _tables():
    k1o = np.concatenate([np.arange(0, 128, 2), np.arange(1, 128, 2)])
    n1 = np.arange(128)
    f = []
    for n2 in range(4):
        e = np.exp(-2j * np.pi * np.outer(k1o + 0.5, 4 * n1 + n2) / M)
        f.append(np.concatenate([e.real, e.imag], 0))
    f = np.stack(f)
    f = f.reshape(4, 2, 16, 8, 128).transpose(0, 2, 1, 3, 4).reshape(4, 256, 128)
    gi = np.transpose(f, (0, 2, 1)) * (2.0 / M)
    gi = gi.reshape(4, 128, 2, 128).transpose(0, 2, 1, 3)
    return _pack_rows(f), _pack_rows(gi)


_F1, _G1 = _tables()


def _dft4(x, sign):
    (r0, i0), (r1, i1), (r2, i2), (r3, i3) = x
    ar, ai = r0 + r2, i0 + i2
    br, bi = r0 - r2, i0 - i2
    cr, ci = r1 + r3, i1 + i3
    dr, di = r1 - r3, i1 - i3
    o0 = (ar + cr, ai + ci)
    o2 = (ar - cr, ai - ci)
    op = (br - di, bi + dr)
    om = (br + di, bi - dr)
    return [o0, op, o2, om] if sign > 0 else [o0, om, o2, op]


def _half_dft4(x, odd_k2):
    (r0, i0), (r1, i1), (r2, i2), (r3, i3) = x
    if not odd_k2:
        ar, ai = r0 + r2, i0 + i2
        cr, ci = r1 + r3, i1 + i3
        return [(ar + cr, ai + ci), (ar - cr, ai - ci)]
    br, bi = r0 - r2, i0 - i2
    dr, di = r1 - r3, i1 - i3
    return [(br + di, bi - dr), (br - di, bi + dr)]


def _kernel(q_hbm, ak_hbm, av_hbm, af_hbm, bk_hbm, bv_hbm, bf_hbm,
            ash_ref, ad_ref, bsh_ref, bd_ref, gw_ref, f1_ref, g1_ref,
            o_hbm,
            q_buf, k_buf, v_buf, f_buf, o_buf,
            k32, kv32, kt32, sp0, sp1, rr0, rr1, ya0, ya1, ya2, ya3, ya4, yb0, yb1, yb2, yb3, yb4, gate, par,
            sem_in, sem_q, sem_out, zref, rb0, rb1):
    rb_ = (rb0, rb1)
    k_h = (ak_hbm, bk_hbm)
    v_h = (av_hbm, bv_hbm)
    f_h = (af_hbm, bf_hbm)
    sh = (ash_ref, bsh_ref)
    dd = (ad_ref, bd_ref)
    sp, rr = (sp0, sp1), (rr0, rr1)
    yy = ((ya0, ya1, ya2, ya3, ya4), (yb0, yb1, yb2, yb3, yb4))

    def in_copies(g, m):
        c0 = pl.multiple_of(g * 128, 128)
        it = g * 2 + m
        return (
            pltpu.make_async_copy(f_h[m].at[pl.ds(c0, 128), :], f_buf.at[it], sem_in.at[it, 0]),
            pltpu.make_async_copy(k_h[m].at[:, pl.ds(c0, 128)], k_buf.at[it], sem_in.at[it, 1]),
            pltpu.make_async_copy(v_h[m].at[:, pl.ds(c0, 128)], v_buf.at[it], sem_in.at[it, 2]),
        )

    def q_copy(g):
        return pltpu.make_async_copy(q_hbm.at[:, pl.ds(g * 128, 128)], q_buf.at[g], sem_q.at[g])

    def o_copy(g, i):
        rows = pl.ds(512 * i, 512)
        return pltpu.make_async_copy(o_buf.at[g, rows, :], o_hbm.at[rows, pl.ds(g * 128, 128)], sem_out.at[g, i])

    last, lastk = [None], [None]
    def tr_block(it, c):
        blk = f_buf[it, :, c * 128:(c + 1) * 128].astype(F32)
        bt = blk.T
        kt32[c * 128:(c + 1) * 128, :] = bt
        lastk[0] = bt[120:128]

    def conv_block(it, c):
        rows = pl.ds(128 * c, 128)
        acc = None
        for t in range(4):
            x = k32[pl.ds(8 + 128 * c - t, 128), :]
            wt = jnp.broadcast_to(par[it, t][0:1, :], (128, 128))
            acc = x * wt if acc is None else acc + x * wt
        kvv = acc * v_buf[it, rows, :].astype(F32)
        kv32[rows, :] = kvv
        last[0] = kvv[112:128, :]

    def unpack_block(it, c):
        k32[pl.ds(8 + 128 * c, 128), :] = k_buf[it, pl.ds(128 * c, 128), :].astype(F32)

    def fwd_chunk(src, dst, off, j):
        outs = []
        for n2 in range(4):
            w = src[pl.ds(512 * j + n2, 128, stride=4), :].astype(BF16)
            outs.append(jnp.dot(pltpu.bitcast(f1_ref[n2], BF16), w, preferred_element_type=F32))
        if not FD:
            for n2 in range(4):
                dst[off + j * 4 + n2] = outs[n2]
            return
        for r in range(16):
            x = _dft4([(o[16 * r:16 * r + 8], o[16 * r + 8:16 * r + 16]) for o in outs], -1)
            for k2 in range(4):
                dst[off + j * 4 + k2, pl.ds(16 * r, 8), :] = x[k2][0]
                dst[off + j * 4 + k2, pl.ds(16 * r + 8, 8), :] = x[k2][1]

    def inv_chunk(it, m, i):
        ydst = yy[m][it // 2]
        if not ID:
            for n2 in range(4):
                p = i * 4 + n2
                y = (jnp.dot(pltpu.bitcast(g1_ref[n2, 0], BF16), rb_[m][p, 0:128, :], preferred_element_type=F32)
                     + jnp.dot(pltpu.bitcast(g1_ref[n2, 1], BF16), rb_[m][p, 128:256, :], preferred_element_type=F32))
                ydst[pl.ds(512 * i + n2, 128, stride=4), :] = y
            return
        parts = [[] for _ in range(4)]
        for r in range(16):
            y = [(rr[m][i * 4 + k2, pl.ds(16 * r, 8), :], rr[m][i * 4 + k2, pl.ds(16 * r + 8, 8), :])
                 for k2 in range(4)]
            x = _dft4(y, +1)
            for n2 in range(4):
                parts[n2].append(jnp.concatenate([x[n2][0], x[n2][1]], axis=0).astype(BF16))
        for n2 in range(4):
            ra = jnp.concatenate(parts[n2][:8], axis=0)
            rb = jnp.concatenate(parts[n2][8:], axis=0)
            y = (jnp.dot(pltpu.bitcast(g1_ref[n2, 0], BF16), ra, preferred_element_type=F32)
                 + jnp.dot(pltpu.bitcast(g1_ref[n2, 1], BF16), rb, preferred_element_type=F32))
            ydst[pl.ds(512 * i + n2, 128, stride=4), :] = y

    def spec_row(it, m, r):
        re = pl.ds(16 * r, 8)
        im = pl.ds(16 * r + 8, 8)
        odd = r >= 8
        dvec = par[it, 4]
        s_ = sp[m]

        def ld(idx):
            return (s_[idx, re, :], s_[idx, im, :])

        def kprime(kk):
            kp = [(kk[0][0] + dvec, kk[0][1])]
            for mm in range(1, 4):
                pr, pi_ = kk[mm - 1]
                if odd:
                    kp.append((kk[mm][0] + pi_, kk[mm][1] - pr))
                else:
                    kp.append((kk[mm][0] - pi_, kk[mm][1] + pr))
            return kp

        def conv(uu, kp):
            out = []
            for i in range(4):
                yr = yi = None
                for j in range(i + 1):
                    ur, ui = uu[j]
                    kr, ki = kp[i - j]
                    pr = ur * kr - ui * ki
                    pi_ = ur * ki + ui * kr
                    yr = pr if yr is None else yr + pr
                    yi = pi_ if yi is None else yi + pi_
                out.append((yr, yi))
            return out

        Y = [[None] * 4 for _ in range(4)]
        if FD:
            for k2 in range(4):
                yo = conv([ld(mm * 4 + k2) for mm in range(4)],
                          kprime([ld(16 + mm * 4 + k2) for mm in range(4)]))
                for i in range(4):
                    Y[i][k2] = yo[i]
                    if ID:
                        rr[m][i * 4 + k2, re, :] = yo[i][0]
                        rr[m][i * 4 + k2, im, :] = yo[i][1]
        else:
            for ok in (False, True):
                k2s = (1, 3) if ok else (0, 2)
                kk = [_half_dft4([ld(16 + mm * 4 + n2) for n2 in range(4)], ok) for mm in range(4)]
                kp = [kprime([kk[mm][a] for mm in range(4)]) for a in range(2)]
                for j in range(4):
                    uu = _half_dft4([ld(j * 4 + n2) for n2 in range(4)], ok)
                    for i in range(j, 4):
                        for a in range(2):
                            ur, ui = uu[a]
                            kr, ki = kp[a][i - j]
                            pr = ur * kr - ui * ki
                            pi_ = ur * ki + ui * kr
                            cur = Y[i][k2s[a]]
                            Y[i][k2s[a]] = (pr, pi_) if cur is None else (cur[0] + pr, cur[1] + pi_)
                if ID:
                    for i in range(4):
                        for a in range(2):
                            rr[m][i * 4 + k2s[a], re, :] = Y[i][k2s[a]][0]
                            rr[m][i * 4 + k2s[a], im, :] = Y[i][k2s[a]][1]
        if not ID:
            for i in range(4):
                ro = _dft4(Y[i], +1)
                for n2 in range(4):
                    rb_[m][i * 4 + n2, pl.ds(16 * r, 16), :] = jnp.concatenate(
                        [ro[n2][0], ro[n2][1]], axis=0).astype(BF16)

    def out_block(g, c):
        rows = pl.ds(128 * c, 128)
        ya = yy[0][g][rows, :]
        yb = yy[1][g][rows, :]
        o_buf[g, rows, :] = (q_buf[g, rows, :].astype(F32) * (yb + gate[rows, :] * (ya - yb))).astype(BF16)

    def gate_block(c):
        rows = pl.ds(128 * c, 128)
        gw = gw_ref[...].astype(F32)[None, :]
        acc = None
        for g in range(NG):
            t = q_buf[g, rows, :].astype(F32) * gw[:, g * 128:(g + 1) * 128]
            acc = t if acc is None else acc + t
        z = jnp.sum(acc, axis=1, keepdims=True)
        gate[rows, :] = jnp.broadcast_to(0.5 * jnp.tanh(0.5 * z) + 0.5, (128, 128))

    def slot(d=None, m1=None, m2=None, out_g=None, do_gate=False, part='CB', tag=''):
        nm = "S_" + ("D" if d else "") + ("M" if m1 else "") + ("E" if m2 else "") + ("F" if out_g is not None else "") + ("G" if do_gate else "") + tag
        if NOSCOPE:
            slot_(d, m1, m2, out_g, do_gate, part)
            return
        with jax.named_scope(nm):
            slot_(d, m1, m2, out_g, do_gate, part)

    def slot_(d, m1, m2, out_g, do_gate, part):
        def prep(c):
            if m1 is not None and c < 16:
                if 'C' in part:
                    tr_block(m1[0], c)
                if 'B' in part:
                    unpack_block(m1[0], c)
                    conv_block(m1[0], c)
        lag = m2 is not None and out_g is not None and m2[0] == 2 * out_g + 1
        edep = ED and m2 is not None and m1 is not None
        if edep:
            for i in range(4):
                for e in range(4):
                    prep(4 * i + e)
                if ID:
                    rr[m2[1]][zref[0] - 16, 0:16, :] = last[0]
                else:
                    rb_[m2[1]][zref[0] - 16, 0:16, :] = last[0].astype(BF16)
                inv_chunk(m2[0], m2[1], i)
        elif m2 is not None and EF:
            for i in range(4):
                inv_chunk(m2[0], m2[1], i)
        if not edep:
            for c in range(LEAD):
                prep(c)
        for j in range(4):
            if not edep:
                for e in range(4):
                    prep(4 * j + e + LEAD)
            if m1 is not None and GP and j < 3:
                zs = pl.ds(pl.multiple_of(zref[0] * 64, 8), 8)
                if 'B' in part:
                    kv32[zs, :] = last[0][0:8]
                if 'C' in part:
                    kt32[zs, :] = lastk[0]
            if m1 is not None:
                for which in ('BC' if BC else 'CB'):
                    if which == 'C' and 'C' in part:
                        fwd_chunk(kt32, sp[m1[1]], 16, j)
                    if which == 'B' and 'B' in part:
                        fwd_chunk(kv32, sp[m1[1]], 0, j)
            if m2 is not None and not EF and not edep:
                inv_chunk(m2[0], m2[1], j)
            for q in range(4 * j, 4 * j + 4):
                if d is not None:
                    spec_row(d[0], d[1], q)
                if do_gate:
                    gate_block(q)
                if out_g is not None and (q >= 4 or not lag):
                    c = q - 4 if lag else q
                    out_block(out_g, c)
                    if c % 4 == 3:
                        o_copy(out_g, c // 4).start()
        if out_g is not None:
            if lag:
                for c in range(12, 16):
                    out_block(out_g, c)
                o_copy(out_g, 3).start()

    def start(g, m):
        for c in in_copies(g, m):
            c.start()

    def wait(g, m):
        for c in in_copies(g, m):
            c.wait()

    def between(name, fn):
        if NOWHEN:
            fn()
            return
        with jax.named_scope("W_" + name):
            @pl.when(zref[0] > 0)
            def _():
                fn()

    start(0, 0)
    k32[0:8, :] = jnp.zeros((8, 128), F32)
    zref[0] = 32
    for m in range(2):
        shw = sh[m][...].astype(F32)
        dv = dd[m][...].astype(F32)[None, :]
        for g in range(NG):
            for t in range(4):
                par[g * 2 + m, t] = jnp.broadcast_to(shw[t:t + 1, g * 128:(g + 1) * 128], (8, 128))
            par[g * 2 + m, 4] = jnp.broadcast_to(dv[:, g * 128:(g + 1) * 128], (8, 128))

    def wstart(name, before=(), waits=(), after=()):
        def cps(x):
            if x[0] == 'i':
                return in_copies(x[1] // 2, x[1] % 2)
            if x[0] == 'f':
                return in_copies(x[1] // 2, x[1] % 2)[:1]
            if x[0] == 'u':
                return in_copies(x[1] // 2, x[1] % 2)[1:]
            return (q_copy(x[1]),)

        def fn():
            for x in before:
                for c in cps(x):
                    c.start()
            for x in waits:
                for c in cps(x):
                    c.wait()
            for x in after:
                for c in cps(x):
                    c.start()
        between(name, fn)

    wstart("0", waits=[('f', 0)], after=[('i', 1)])
    if not EXP:
        slot(m1=(0, 0), part='C', tag='0a')
    wstart("0b", waits=[('u', 0)])
    if not EXP:
        slot(m1=(0, 0), part='B', tag='0b')
    QS = {2: [0], 3: [1, 2], 4: [3], 5: [4]}
    FS = {7: 0, 8: 1, 9: 2, 10: 3}
    for t in (range(1, 10) if not EXP else EXP):
        before, after = [], []
        if t == 1:
            before = [('i', 2)]
        elif t in (2, 3, 4, 5):
            after = [('i', t + 1)]
        elif t == 6:
            after = [('i', 7), ('i', 8)]
        elif t + 2 <= 9:
            after = [('i', t + 2)]
        after += [('q', g) for g in QS.get(t, [])]
        waits = [('i', t)] + ([('q', g) for g in range(NG)] if t == 6 else [])
        if SPLIT or t in SPL:
            slot(d=(t - 1, (t - 1) % 2), tag='%d' % t)
            wstart("%d" % t, before, waits, after)
            slot(m1=(t, t % 2), m2=(t - 2, t % 2) if t >= 2 else None,
                 out_g=FS.get(t), do_gate=(t == 6), tag='%d' % t)
        else:
            wstart("%d" % t, before, waits, after)
            slot(d=(t - 1, (t - 1) % 2), m1=(t, t % 2), m2=(t - 2, t % 2) if t >= 2 else None,
                 out_g=FS.get(t), do_gate=(t == 6), tag='%d' % t)
    if not EXP:
        slot(d=(9, 1), m2=(8, 0), out_g=FS.get(10), tag='10')
    slot(m2=(9, 1), out_g=NG - 1, tag='11')
    with jax.named_scope("W_out"):
        for g in range(NG):
            for i in range(4):
                o_copy(g, i).wait()


@jax.jit
def pallas_gated_mix__ssm_conv_h3__ssm_conv_h3__prompt_kernel(
        A_q, A_k, A_v, A_shift_k, A_ssm_k, A_ssm_D,
        B_q, B_k, B_v, B_shift_k, B_ssm_k, B_ssm_D, gate_w):
    hbm = pl.BlockSpec(memory_space=pl.ANY)
    vm = pl.BlockSpec(memory_space=pltpu.VMEM)
    sq = lambda x: x.reshape(S, D)
    out = pl.pallas_call(
        _kernel,
        out_shape=jax.ShapeDtypeStruct((S, D), BF16),
        in_specs=[hbm] * 7 + [vm] * 7,
        out_specs=hbm,
        scratch_shapes=[
            pltpu.VMEM((NG, S, 128), BF16),
            pltpu.VMEM((2 * NG, S, 128), BF16),
            pltpu.VMEM((2 * NG, S, 128), BF16),
            pltpu.VMEM((2 * NG, 128, S), BF16),
            pltpu.VMEM((NG, S, 128), BF16),
            pltpu.VMEM((S + 8, 128), F32),
            pltpu.VMEM((S + 8, 128), F32),
            pltpu.VMEM((S + 8, 128), F32),
            pltpu.VMEM((32, 256, 128), F32),
            pltpu.VMEM((32, 256, 128), F32),
            pltpu.VMEM((17, 256, 128), F32),
            pltpu.VMEM((17, 256, 128), F32),
            *[pltpu.VMEM((S, 128), F32) for _ in range(2 * NG)],
            pltpu.VMEM((S, 128), F32),
            pltpu.VMEM((2 * NG, 5, 8, 128), F32),
            pltpu.SemaphoreType.DMA((2 * NG, 3)),
            pltpu.SemaphoreType.DMA((NG,)),
            pltpu.SemaphoreType.DMA((NG, 4)),
            pltpu.SMEM((1,), jnp.int32),
            pltpu.VMEM((17, 256, 128), BF16),
            pltpu.VMEM((17, 256, 128), BF16),
        ],
        compiler_params=pltpu.CompilerParams(vmem_limit_bytes=100 * 1024 * 1024),
    )(sq(A_q), sq(A_k), sq(A_v), A_ssm_k, sq(B_k), sq(B_v), B_ssm_k,
      A_shift_k.T, A_ssm_D, B_shift_k.T, B_ssm_D, gate_w, _F1, _G1)
    return out.reshape(1, S, D)
```

```python
import numpy as np
import jax
import jax.numpy as jnp
import jax.experimental.pallas as pl
import jax.experimental.pallas.tpu as pltpu
import ml_dtypes

S = 2048
D = 640
NG = 5
M = 1024
F32 = jnp.float32
BF16 = jnp.bfloat16
EF = 1
FD = 1
ID = 0
ED = 0
SPLIT = 0
LEAD = 4
BC = 0
EXP = []
NOWHEN = 0
NOSCOPE = 0
SPL = [1]
GP = 0
FLAGS = {'XLA_TPU_EVENLY_DISTRIBUTE_CRITICAL_NODES': True}
GM = 1


def _pack_rows(x):
    b = np.ascontiguousarray(x).astype(ml_dtypes.bfloat16).view(np.uint16).astype(np.uint32)
    return b[..., 0::2, :] | (b[..., 1::2, :] << 16)


def _tables():
    k1o = np.concatenate([np.arange(0, 128, 2), np.arange(1, 128, 2)])
    n1 = np.arange(128)
    f = []
    for n2 in range(4):
        e = np.exp(-2j * np.pi * np.outer(k1o + 0.5, 4 * n1 + n2) / M)
        f.append(np.concatenate([e.real, e.imag], 0))
    f = np.stack(f)
    f = f.reshape(4, 2, 16, 8, 128).transpose(0, 2, 1, 3, 4).reshape(4, 256, 128)
    gi = np.transpose(f, (0, 2, 1)) * (2.0 / M)
    gi = gi.reshape(4, 128, 2, 128).transpose(0, 2, 1, 3)
    return _pack_rows(f), _pack_rows(gi)


_F1, _G1 = _tables()


def _dft4(x, sign):
    (r0, i0), (r1, i1), (r2, i2), (r3, i3) = x
    ar, ai = r0 + r2, i0 + i2
    br, bi = r0 - r2, i0 - i2
    cr, ci = r1 + r3, i1 + i3
    dr, di = r1 - r3, i1 - i3
    o0 = (ar + cr, ai + ci)
    o2 = (ar - cr, ai - ci)
    op = (br - di, bi + dr)
    om = (br + di, bi - dr)
    return [o0, op, o2, om] if sign > 0 else [o0, om, o2, op]


def _half_dft4(x, odd_k2):
    (r0, i0), (r1, i1), (r2, i2), (r3, i3) = x
    if not odd_k2:
        ar, ai = r0 + r2, i0 + i2
        cr, ci = r1 + r3, i1 + i3
        return [(ar + cr, ai + ci), (ar - cr, ai - ci)]
    br, bi = r0 - r2, i0 - i2
    dr, di = r1 - r3, i1 - i3
    return [(br + di, bi - dr), (br - di, bi + dr)]


def _kernel(q_hbm, ak_hbm, av_hbm, af_hbm, bk_hbm, bv_hbm, bf_hbm,
            ash_ref, ad_ref, bsh_ref, bd_ref, gw_ref, f1_hbm, g1_hbm,
            o_hbm, f1_ref, g1_ref, sem_t,
            q_buf, k_buf, v_buf, f_buf, o_buf,
            k32, kv32, kt32, sp0, sp1, rr0, rr1, ya0, ya1, ya2, ya3, ya4, yb0, yb1, yb2, yb3, yb4, gate, par,
            sem_in, sem_q, sem_out, zref, rb0, rb1):
    rb_ = (rb0, rb1)
    k_h = (ak_hbm, bk_hbm)
    v_h = (av_hbm, bv_hbm)
    f_h = (af_hbm, bf_hbm)
    sh = (ash_ref, bsh_ref)
    dd = (ad_ref, bd_ref)
    sp, rr = (sp0, sp1), (rr0, rr1)
    yy = ((ya0, ya1, ya2, ya3, ya4), (yb0, yb1, yb2, yb3, yb4))

    def in_copies(g, m, which='fkv'):
        c0 = g * 128
        it = g * 2 + m
        mk = {
            'f': lambda: pltpu.make_async_copy(f_h[m].at[pl.ds(c0, 128), :], f_buf.at[it], sem_in.at[it, 0]),
            'k': lambda: pltpu.make_async_copy(k_h[m].at[:, pl.ds(c0, 128)], k_buf.at[it], sem_in.at[it, 1]),
            'v': lambda: pltpu.make_async_copy(v_h[m].at[:, pl.ds(c0, 128)], v_buf.at[it], sem_in.at[it, 2]),
        }
        return tuple(mk[w]() for w in which)

    def q_copy(g):
        return pltpu.make_async_copy(q_hbm.at[:, pl.ds(g * 128, 128)], q_buf.at[g], sem_q.at[g])

    def o_copy(g, i):
        rows = pl.ds(512 * i, 512)
        return pltpu.make_async_copy(o_buf.at[g, rows, :], o_hbm.at[rows, pl.ds(g * 128, 128)], sem_out.at[g, i])

    last, lastk = [None], [None]
    def tr_block(it, c):
        blk = f_buf[it, :, c * 128:(c + 1) * 128].astype(F32)
        bt = blk.T
        kt32[c * 128:(c + 1) * 128, :] = bt
        lastk[0] = bt[120:128]

    def conv_block(it, c):
        rows = pl.ds(128 * c, 128)
        acc = None
        for t in range(4):
            x = k32[pl.ds(8 + 128 * c - t, 128), :]
            wt = jnp.broadcast_to(par[it, t][0:1, :], (128, 128))
            acc = x * wt if acc is None else acc + x * wt
        kvv = acc * v_buf[it, rows, :].astype(F32)
        kv32[rows, :] = kvv
        last[0] = kvv[112:128, :]

    def unpack_block(it, c):
        k32[pl.ds(8 + 128 * c, 128), :] = k_buf[it, pl.ds(128 * c, 128), :].astype(F32)

    def fwd_chunk(src, dst, off, j):
        outs = []
        for n2 in range(4):
            w = src[pl.ds(512 * j + n2, 128, stride=4), :].astype(BF16)
            outs.append(jnp.dot(pltpu.bitcast(f1_ref[n2], BF16), w, preferred_element_type=F32))
        if not FD:
            for n2 in range(4):
                dst[off + j * 4 + n2] = outs[n2]
            return
        for r in range(16):
            x = _dft4([(o[16 * r:16 * r + 8], o[16 * r + 8:16 * r + 16]) for o in outs], -1)
            for k2 in range(4):
                dst[off + j * 4 + k2, pl.ds(16 * r, 8), :] = x[k2][0]
                dst[off + j * 4 + k2, pl.ds(16 * r + 8, 8), :] = x[k2][1]

    def inv_chunk(it, m, i):
        ydst = yy[m][it // 2]
        if not ID:
            for n2 in range(4):
                p = i * 4 + n2
                y = (jnp.dot(pltpu.bitcast(g1_ref[n2, 0], BF16), rb_[m][p, 0:128, :], preferred_element_type=F32)
                     + jnp.dot(pltpu.bitcast(g1_ref[n2, 1], BF16), rb_[m][p, 128:256, :], preferred_element_type=F32))
                ydst[pl.ds(512 * i + n2, 128, stride=4), :] = y
            return
        parts = [[] for _ in range(4)]
        for r in range(16):
            y = [(rr[m][i * 4 + k2, pl.ds(16 * r, 8), :], rr[m][i * 4 + k2, pl.ds(16 * r + 8, 8), :])
                 for k2 in range(4)]
            x = _dft4(y, +1)
            for n2 in range(4):
                parts[n2].append(jnp.concatenate([x[n2][0], x[n2][1]], axis=0).astype(BF16))
        for n2 in range(4):
            ra = jnp.concatenate(parts[n2][:8], axis=0)
            rb = jnp.concatenate(parts[n2][8:], axis=0)
            y = (jnp.dot(pltpu.bitcast(g1_ref[n2, 0], BF16), ra, preferred_element_type=F32)
                 + jnp.dot(pltpu.bitcast(g1_ref[n2, 1], BF16), rb, preferred_element_type=F32))
            ydst[pl.ds(512 * i + n2, 128, stride=4), :] = y

    def spec_row(it, m, r):
        re = pl.ds(16 * r, 8)
        im = pl.ds(16 * r + 8, 8)
        odd = r >= 8
        dvec = par[it, 4]
        s_ = sp[m]

        def ld(idx):
            return (s_[idx, re, :], s_[idx, im, :])

        def kprime(kk):
            kp = [(kk[0][0] + dvec, kk[0][1])]
            for mm in range(1, 4):
                pr, pi_ = kk[mm - 1]
                if odd:
                    kp.append((kk[mm][0] + pi_, kk[mm][1] - pr))
                else:
                    kp.append((kk[mm][0] - pi_, kk[mm][1] + pr))
            return kp

        def conv(uu, kp):
            out = []
            for i in range(4):
                yr = yi = None
                for j in range(i + 1):
                    ur, ui = uu[j]
                    kr, ki = kp[i - j]
                    pr = ur * kr - ui * ki
                    pi_ = ur * ki + ui * kr
                    yr = pr if yr is None else yr + pr
                    yi = pi_ if yi is None else yi + pi_
                out.append((yr, yi))
            return out

        Y = [[None] * 4 for _ in range(4)]
        if FD:
            for k2 in range(4):
                yo = conv([ld(mm * 4 + k2) for mm in range(4)],
                          kprime([ld(16 + mm * 4 + k2) for mm in range(4)]))
                for i in range(4):
                    Y[i][k2] = yo[i]
                    if ID:
                        rr[m][i * 4 + k2, re, :] = yo[i][0]
                        rr[m][i * 4 + k2, im, :] = yo[i][1]
        else:
            for ok in (False, True):
                k2s = (1, 3) if ok else (0, 2)
                kk = [_half_dft4([ld(16 + mm * 4 + n2) for n2 in range(4)], ok) for mm in range(4)]
                kp = [kprime([kk[mm][a] for mm in range(4)]) for a in range(2)]
                for j in range(4):
                    uu = _half_dft4([ld(j * 4 + n2) for n2 in range(4)], ok)
                    for i in range(j, 4):
                        for a in range(2):
                            ur, ui = uu[a]
                            kr, ki = kp[a][i - j]
                            pr = ur * kr - ui * ki
                            pi_ = ur * ki + ui * kr
                            cur = Y[i][k2s[a]]
                            Y[i][k2s[a]] = (pr, pi_) if cur is None else (cur[0] + pr, cur[1] + pi_)
                if ID:
                    for i in range(4):
                        for a in range(2):
                            rr[m][i * 4 + k2s[a], re, :] = Y[i][k2s[a]][0]
                            rr[m][i * 4 + k2s[a], im, :] = Y[i][k2s[a]][1]
        if not ID:
            for i in range(4):
                ro = _dft4(Y[i], +1)
                for n2 in range(4):
                    rb_[m][i * 4 + n2, pl.ds(16 * r, 16), :] = jnp.concatenate(
                        [ro[n2][0], ro[n2][1]], axis=0).astype(BF16)

    def out_block(g, c):
        rows = pl.ds(128 * c, 128)
        ya = yy[0][g][rows, :]
        yb = yy[1][g][rows, :]
        o_buf[g, rows, :] = (q_buf[g, rows, :].astype(F32) * (yb + gate[rows, :] * (ya - yb))).astype(BF16)

    def gate_block(c):
        rows = pl.ds(128 * c, 128)
        gw = gw_ref[...].astype(F32)[None, :]
        acc = None
        for g in range(NG):
            t = q_buf[g, rows, :].astype(F32) * gw[:, g * 128:(g + 1) * 128]
            acc = t if acc is None else acc + t
        z = jnp.sum(acc, axis=1, keepdims=True)
        gate[rows, :] = jnp.broadcast_to(0.5 * jnp.tanh(0.5 * z) + 0.5, (128, 128))

    def slot(d=None, m1=None, m2=None, out_g=None, do_gate=False, part='CB', tag=''):
        nm = "S_" + ("D" if d else "") + ("M" if m1 else "") + ("E" if m2 else "") + ("F" if out_g is not None else "") + ("G" if do_gate else "") + tag
        if NOSCOPE:
            slot_(d, m1, m2, out_g, do_gate, part)
            return
        with jax.named_scope(nm):
            slot_(d, m1, m2, out_g, do_gate, part)

    def slot_(d, m1, m2, out_g, do_gate, part):
        def prep(c):
            if m1 is not None and c < 16:
                if 'C' in part:
                    tr_block(m1[0], c)
                if 'B' in part:
                    unpack_block(m1[0], c)
                    conv_block(m1[0], c)
        lag = m2 is not None and out_g is not None and m2[0] == 2 * out_g + 1
        edep = ED and m2 is not None and m1 is not None
        if edep:
            for i in range(4):
                for e in range(4):
                    prep(4 * i + e)
                if ID:
                    rr[m2[1]][zref[0] - 16, 0:16, :] = last[0]
                else:
                    rb_[m2[1]][zref[0] - 16, 0:16, :] = last[0].astype(BF16)
                inv_chunk(m2[0], m2[1], i)
        elif m2 is not None and EF:
            for i in range(4):
                inv_chunk(m2[0], m2[1], i)
        if not edep:
            for c in range(LEAD):
                prep(c)
        for j in range(4):
            if not edep:
                for e in range(4):
                    prep(4 * j + e + LEAD)
            if m1 is not None and GP and j < 3:
                zs = pl.ds(pl.multiple_of(zref[0] * 64, 8), 8)
                if 'B' in part:
                    kv32[zs, :] = last[0][0:8]
                if 'C' in part:
                    kt32[zs, :] = lastk[0]
            if m1 is not None:
                for which in ('BC' if BC else 'CB'):
                    if which == 'C' and 'C' in part:
                        fwd_chunk(kt32, sp[m1[1]], 16, j)
                    if which == 'B' and 'B' in part:
                        fwd_chunk(kv32, sp[m1[1]], 0, j)
            if m2 is not None and not EF and not edep:
                inv_chunk(m2[0], m2[1], j)
            for q in range(4 * j, 4 * j + 4):
                if d is not None:
                    spec_row(d[0], d[1], q)
                if do_gate:
                    gate_block(q)
                if out_g is not None and (q >= 4 or not lag):
                    c = q - 4 if lag else q
                    out_block(out_g, c)
                    if c % 4 == 3:
                        o_copy(out_g, c // 4).start()
        if out_g is not None:
            if lag:
                for c in range(12, 16):
                    out_block(out_g, c)
                o_copy(out_g, 3).start()

    def start(g, m):
        for c in in_copies(g, m):
            c.start()

    def wait(g, m):
        for c in in_copies(g, m):
            c.wait()

    def between(name, fn):
        if NOWHEN:
            fn()
            return
        with jax.named_scope("W_" + name):
            @pl.when(zref[0] > 0)
            def _():
                fn()

    pltpu.make_async_copy(f1_hbm, f1_ref, sem_t.at[0]).start()
    start(0, 0)
    k32[0:8, :] = jnp.zeros((8, 128), F32)
    zref[0] = 32
    for m in range(2):
        shw = sh[m][...].astype(F32)
        dv = dd[m][...].astype(F32)[None, :]
        for g in range(NG):
            for t in range(4):
                par[g * 2 + m, t] = jnp.broadcast_to(shw[t:t + 1, g * 128:(g + 1) * 128], (8, 128))
            par[g * 2 + m, 4] = jnp.broadcast_to(dv[:, g * 128:(g + 1) * 128], (8, 128))

    def wstart(name, before=(), waits=(), after=()):
        def cps(x):
            if x[0] == 'i':
                return in_copies(x[1] // 2, x[1] % 2)
            if x[0] == 'f':
                return in_copies(x[1] // 2, x[1] % 2, 'f')
            if x[0] == 'u':
                return in_copies(x[1] // 2, x[1] % 2, 'kv')
            if x[0] == 't':
                return (pltpu.make_async_copy((f1_hbm, g1_hbm)[x[1]], (f1_ref, g1_ref)[x[1]], sem_t.at[x[1]]),)
            return (q_copy(x[1]),)

        def fn():
            for x in before:
                for c in cps(x):
                    c.start()
            for x in waits:
                for c in cps(x):
                    c.wait()
            for x in after:
                for c in cps(x):
                    c.start()
        between(name, fn)

    wstart("0", waits=[('f', 0), ('t', 0)], after=[('i', 1)])
    if not EXP:
        slot(m1=(0, 0), part='C', tag='0a')
    wstart("0b", waits=[('u', 0)], after=[('i', 2), ('t', 1)])
    if not EXP:
        slot(m1=(0, 0), part='B', tag='0b')
    QS = {2: [0], 3: [1, 2], 4: [3], 5: [4]}
    FS = {7: 0, 8: 1, 9: 2, 10: 3}
    for t in (range(1, 10) if not EXP else EXP):
        before, after = [], []
        if t + 2 <= 9:
            after = [('i', t + 2)]
        after += [('q', g) for g in QS.get(t, [])]
        waits = [('i', t)] + ([('t', 1)] if t == 2 else []) + ([('q', g) for g in range(NG)] if t == 6 else [])
        if SPLIT or t in SPL:
            slot(d=(t - 1, (t - 1) % 2), tag='%d' % t)
            wstart("%d" % t, before, waits, after)
            slot(m1=(t, t % 2), m2=(t - 2, t % 2) if t >= 2 else None,
                 out_g=FS.get(t), do_gate=(t == 6), tag='%d' % t)
        else:
            wstart("%d" % t, before, waits, after)
            slot(d=(t - 1, (t - 1) % 2), m1=(t, t % 2), m2=(t - 2, t % 2) if t >= 2 else None,
                 out_g=FS.get(t), do_gate=(t == 6), tag='%d' % t)
    if not EXP:
        slot(d=(9, 1), m2=(8, 0), out_g=FS.get(10), tag='10')
    slot(m2=(9, 1), out_g=NG - 1, tag='11')
    with jax.named_scope("W_out"):
        for g in range(NG):
            for i in range(4):
                o_copy(g, i).wait()


@jax.jit
def pallas_gated_mix__ssm_conv_h3__ssm_conv_h3__prompt_kernel(
        A_q, A_k, A_v, A_shift_k, A_ssm_k, A_ssm_D,
        B_q, B_k, B_v, B_shift_k, B_ssm_k, B_ssm_D, gate_w):
    hbm = pl.BlockSpec(memory_space=pl.ANY)
    vm = pl.BlockSpec(memory_space=pltpu.VMEM)
    sq = lambda x: x.reshape(S, D)
    out = pl.pallas_call(
        _kernel,
        out_shape=jax.ShapeDtypeStruct((S, D), BF16),
        in_specs=[hbm] * 7 + [vm] * 5 + [hbm] * 2,
        out_specs=hbm,
        scratch_shapes=[
            pltpu.VMEM((4, 128, 128), jnp.uint32),
            pltpu.VMEM((4, 2, 64, 128), jnp.uint32),
            pltpu.SemaphoreType.DMA((2,)),
            pltpu.VMEM((NG, S, 128), BF16),
            pltpu.VMEM((2 * NG, S, 128), BF16),
            pltpu.VMEM((2 * NG, S, 128), BF16),
            pltpu.VMEM((2 * NG, 128, S), BF16),
            pltpu.VMEM((NG, S, 128), BF16),
            pltpu.VMEM((S + 8, 128), F32),
            pltpu.VMEM((S + 8, 128), F32),
            pltpu.VMEM((S + 8, 128), F32),
            pltpu.VMEM((32, 256, 128), F32),
            pltpu.VMEM((32, 256, 128), F32),
            pltpu.VMEM((17, 256, 128), F32),
            pltpu.VMEM((17, 256, 128), F32),
            *[pltpu.VMEM((S, 128), F32) for _ in range(2 * NG)],
            pltpu.VMEM((S, 128), F32),
            pltpu.VMEM((2 * NG, 5, 8, 128), F32),
            pltpu.SemaphoreType.DMA((2 * NG, 3)),
            pltpu.SemaphoreType.DMA((NG,)),
            pltpu.SemaphoreType.DMA((NG, 4)),
            pltpu.SMEM((1,), jnp.int32),
            pltpu.VMEM((17, 256, 128), BF16),
            pltpu.VMEM((17, 256, 128), BF16),
        ],
        compiler_params=pltpu.CompilerParams(vmem_limit_bytes=100 * 1024 * 1024, flags=FLAGS),
    )(sq(A_q), sq(A_k), sq(A_v), A_ssm_k, sq(B_k), sq(B_v), B_ssm_k,
      A_shift_k.T, A_ssm_D, B_shift_k.T, B_ssm_D, gate_w, _F1, _G1)
    return out.reshape(1, S, D)
```

```python
import numpy as np
import jax
import jax.numpy as jnp
import jax.experimental.pallas as pl
import jax.experimental.pallas.tpu as pltpu
import ml_dtypes

S = 2048
D = 640
NG = 5
M = 1024
F32 = jnp.float32
BF16 = jnp.bfloat16
EF = 1
FD = 1
ID = 0
ED = 1
SPLIT = 0
LEAD = 4
BC = 0
EXP = []
NOWHEN = 0
NOSCOPE = 0
SPL = [1]
GP = 0
FLAGS = {'XLA_TPU_EVENLY_DISTRIBUTE_CRITICAL_NODES': True}
GM = 1


def _pack_rows(x):
    b = np.ascontiguousarray(x).astype(ml_dtypes.bfloat16).view(np.uint16).astype(np.uint32)
    return b[..., 0::2, :] | (b[..., 1::2, :] << 16)


def _tables():
    k1o = np.concatenate([np.arange(0, 128, 2), np.arange(1, 128, 2)])
    n1 = np.arange(128)
    f = []
    for n2 in range(4):
        e = np.exp(-2j * np.pi * np.outer(k1o + 0.5, 4 * n1 + n2) / M)
        f.append(np.concatenate([e.real, e.imag], 0))
    f = np.stack(f)
    f = f.reshape(4, 2, 16, 8, 128).transpose(0, 2, 1, 3, 4).reshape(4, 256, 128)
    gi = np.transpose(f, (0, 2, 1)) * (2.0 / M)
    gi = gi.reshape(4, 128, 2, 128).transpose(0, 2, 1, 3)
    return _pack_rows(f), _pack_rows(gi)


_F1, _G1 = _tables()


def _dft4(x, sign):
    (r0, i0), (r1, i1), (r2, i2), (r3, i3) = x
    ar, ai = r0 + r2, i0 + i2
    br, bi = r0 - r2, i0 - i2
    cr, ci = r1 + r3, i1 + i3
    dr, di = r1 - r3, i1 - i3
    o0 = (ar + cr, ai + ci)
    o2 = (ar - cr, ai - ci)
    op = (br - di, bi + dr)
    om = (br + di, bi - dr)
    return [o0, op, o2, om] if sign > 0 else [o0, om, o2, op]


def _half_dft4(x, odd_k2):
    (r0, i0), (r1, i1), (r2, i2), (r3, i3) = x
    if not odd_k2:
        ar, ai = r0 + r2, i0 + i2
        cr, ci = r1 + r3, i1 + i3
        return [(ar + cr, ai + ci), (ar - cr, ai - ci)]
    br, bi = r0 - r2, i0 - i2
    dr, di = r1 - r3, i1 - i3
    return [(br + di, bi - dr), (br - di, bi + dr)]


def _kernel(q_hbm, ak_hbm, av_hbm, af_hbm, bk_hbm, bv_hbm, bf_hbm,
            ash_ref, ad_ref, bsh_ref, bd_ref, gw_ref, f1_hbm, g1_hbm,
            o_hbm, f1_ref, g1_ref, sem_t,
            q_buf, k_buf, v_buf, f_buf, o_buf,
            k32, kv32, kt32, sp0, sp1, rr0, rr1, ya0, ya1, ya2, ya3, ya4, yb0, yb1, yb2, yb3, yb4, gate, par,
            sem_in, sem_q, sem_out, zref, rb0, rb1):
    rb_ = (rb0, rb1)
    k_h = (ak_hbm, bk_hbm)
    v_h = (av_hbm, bv_hbm)
    f_h = (af_hbm, bf_hbm)
    sh = (ash_ref, bsh_ref)
    dd = (ad_ref, bd_ref)
    sp, rr = (sp0, sp1), (rr0, rr1)
    yy = ((ya0, ya1, ya2, ya3, ya4), (yb0, yb1, yb2, yb3, yb4))

    def in_copies(g, m, which='fkv'):
        c0 = g * 128
        it = g * 2 + m
        mk = {
            'f': lambda: pltpu.make_async_copy(f_h[m].at[pl.ds(c0, 128), :], f_buf.at[it], sem_in.at[it, 0]),
            'k': lambda: pltpu.make_async_copy(k_h[m].at[:, pl.ds(c0, 128)], k_buf.at[it], sem_in.at[it, 1]),
            'v': lambda: pltpu.make_async_copy(v_h[m].at[:, pl.ds(c0, 128)], v_buf.at[it], sem_in.at[it, 2]),
        }
        return tuple(mk[w]() for w in which)

    def q_copy(g):
        return pltpu.make_async_copy(q_hbm.at[:, pl.ds(g * 128, 128)], q_buf.at[g], sem_q.at[g])

    def o_copy(g, i):
        rows = pl.ds(512 * i, 512)
        return pltpu.make_async_copy(o_buf.at[g, rows, :], o_hbm.at[rows, pl.ds(g * 128, 128)], sem_out.at[g, i])

    last, lastk = [None], [None]
    def tr_block(it, c):
        blk = f_buf[it, :, c * 128:(c + 1) * 128].astype(F32)
        bt = blk.T
        kt32[c * 128:(c + 1) * 128, :] = bt
        lastk[0] = bt[120:128]

    def conv_block(it, c):
        rows = pl.ds(128 * c, 128)
        acc = None
        for t in range(4):
            x = k32[pl.ds(8 + 128 * c - t, 128), :]
            wt = jnp.broadcast_to(par[it, t][0:1, :], (128, 128))
            acc = x * wt if acc is None else acc + x * wt
        kvv = acc * v_buf[it, rows, :].astype(F32)
        kv32[rows, :] = kvv
        last[0] = kvv[112:128, :]

    def unpack_block(it, c):
        k32[pl.ds(8 + 128 * c, 128), :] = k_buf[it, pl.ds(128 * c, 128), :].astype(F32)

    def fwd_chunk(src, dst, off, j, dc=None):
        outs = []
        for n2 in range(4):
            w = src[pl.ds(512 * j + n2, 128, stride=4), :].astype(BF16)
            outs.append(jnp.dot(pltpu.bitcast(f1_ref[n2], BF16), w, preferred_element_type=F32))
        if not FD:
            for n2 in range(4):
                dst[off + j * 4 + n2] = outs[n2]
            return
        for r in range(16):
            x = _dft4([(o[16 * r:16 * r + 8], o[16 * r + 8:16 * r + 16]) for o in outs], -1)
            for k2 in range(4):
                dst[off + j * 4 + k2, pl.ds(16 * r, 8), :] = x[k2][0] if dc is None else x[k2][0] + dc
                dst[off + j * 4 + k2, pl.ds(16 * r + 8, 8), :] = x[k2][1]

    def inv_chunk(it, m, i):
        ydst = yy[m][it // 2]
        if not ID:
            for n2 in range(4):
                p = i * 4 + n2
                y = (jnp.dot(pltpu.bitcast(g1_ref[n2, 0], BF16), rb_[m][p, 0:128, :], preferred_element_type=F32)
                     + jnp.dot(pltpu.bitcast(g1_ref[n2, 1], BF16), rb_[m][p, 128:256, :], preferred_element_type=F32))
                ydst[pl.ds(512 * i + n2, 128, stride=4), :] = y
            return
        parts = [[] for _ in range(4)]
        for r in range(16):
            y = [(rr[m][i * 4 + k2, pl.ds(16 * r, 8), :], rr[m][i * 4 + k2, pl.ds(16 * r + 8, 8), :])
                 for k2 in range(4)]
            x = _dft4(y, +1)
            for n2 in range(4):
                parts[n2].append(jnp.concatenate([x[n2][0], x[n2][1]], axis=0).astype(BF16))
        for n2 in range(4):
            ra = jnp.concatenate(parts[n2][:8], axis=0)
            rb = jnp.concatenate(parts[n2][8:], axis=0)
            y = (jnp.dot(pltpu.bitcast(g1_ref[n2, 0], BF16), ra, preferred_element_type=F32)
                 + jnp.dot(pltpu.bitcast(g1_ref[n2, 1], BF16), rb, preferred_element_type=F32))
            ydst[pl.ds(512 * i + n2, 128, stride=4), :] = y

    def spec_row(it, m, r):
        re = pl.ds(16 * r, 8)
        im = pl.ds(16 * r + 8, 8)
        odd = r >= 8
        dvec = par[it, 4]
        s_ = sp[m]

        def ld(idx):
            return (s_[idx, re, :], s_[idx, im, :])

        def kprime(kk):
            kp = [kk[0]]
            for mm in range(1, 4):
                pr, pi_ = kk[mm - 1]
                if odd:
                    kp.append((kk[mm][0] + pi_, kk[mm][1] - pr))
                else:
                    kp.append((kk[mm][0] - pi_, kk[mm][1] + pr))
            return kp

        def conv(uu, kp):
            out = []
            for i in range(4):
                yr = yi = None
                for j in range(i + 1):
                    ur, ui = uu[j]
                    kr, ki = kp[i - j]
                    pr = ur * kr - ui * ki
                    pi_ = ur * ki + ui * kr
                    yr = pr if yr is None else yr + pr
                    yi = pi_ if yi is None else yi + pi_
                out.append((yr, yi))
            return out

        Y = [[None] * 4 for _ in range(4)]
        if FD:
            for k2 in range(4):
                yo = conv([ld(mm * 4 + k2) for mm in range(4)],
                          kprime([ld(16 + mm * 4 + k2) for mm in range(4)]))
                for i in range(4):
                    Y[i][k2] = yo[i]
                    if ID:
                        rr[m][i * 4 + k2, re, :] = yo[i][0]
                        rr[m][i * 4 + k2, im, :] = yo[i][1]
        else:
            for ok in (False, True):
                k2s = (1, 3) if ok else (0, 2)
                kk = [_half_dft4([ld(16 + mm * 4 + n2) for n2 in range(4)], ok) for mm in range(4)]
                kp = [kprime([kk[mm][a] for mm in range(4)]) for a in range(2)]
                for j in range(4):
                    uu = _half_dft4([ld(j * 4 + n2) for n2 in range(4)], ok)
                    for i in range(j, 4):
                        for a in range(2):
                            ur, ui = uu[a]
                            kr, ki = kp[a][i - j]
                            pr = ur * kr - ui * ki
                            pi_ = ur * ki + ui * kr
                            cur = Y[i][k2s[a]]
                            Y[i][k2s[a]] = (pr, pi_) if cur is None else (cur[0] + pr, cur[1] + pi_)
                if ID:
                    for i in range(4):
                        for a in range(2):
                            rr[m][i * 4 + k2s[a], re, :] = Y[i][k2s[a]][0]
                            rr[m][i * 4 + k2s[a], im, :] = Y[i][k2s[a]][1]
        if not ID:
            for i in range(4):
                ro = _dft4(Y[i], +1)
                for n2 in range(4):
                    rb_[m][i * 4 + n2, pl.ds(16 * r, 16), :] = jnp.concatenate(
                        [ro[n2][0], ro[n2][1]], axis=0).astype(BF16)

    def out_block(g, c):
        rows = pl.ds(128 * c, 128)
        ya = yy[0][g][rows, :]
        yb = yy[1][g][rows, :]
        o_buf[g, rows, :] = (q_buf[g, rows, :].astype(F32) * (yb + gate[rows, :] * (ya - yb))).astype(BF16)

    def gate_block(c):
        rows = pl.ds(128 * c, 128)
        gw = gw_ref[...].astype(F32)[None, :]
        acc = None
        for g in range(NG):
            t = q_buf[g, rows, :].astype(F32) * gw[:, g * 128:(g + 1) * 128]
            acc = t if acc is None else acc + t
        z = jnp.sum(acc, axis=1, keepdims=True)
        gate[rows, :] = jnp.broadcast_to(0.5 * jnp.tanh(0.5 * z) + 0.5, (128, 128))

    def slot(d=None, m1=None, m2=None, out_g=None, do_gate=False, part='CB', tag=''):
        nm = "S_" + ("D" if d else "") + ("M" if m1 else "") + ("E" if m2 else "") + ("F" if out_g is not None else "") + ("G" if do_gate else "") + tag
        if NOSCOPE:
            slot_(d, m1, m2, out_g, do_gate, part)
            return
        with jax.named_scope(nm):
            slot_(d, m1, m2, out_g, do_gate, part)

    def slot_(d, m1, m2, out_g, do_gate, part):
        def prep(c):
            if m1 is not None and c < 16:
                if 'C' in part:
                    tr_block(m1[0], c)
                if 'B' in part:
                    unpack_block(m1[0], c)
                    conv_block(m1[0], c)
        lag = m2 is not None and out_g is not None and m2[0] == 2 * out_g + 1
        edep = ED and m2 is not None and m1 is not None
        if edep:
            for i in range(4):
                for e in range(4):
                    prep(4 * i + e)
                if ID:
                    rr[m2[1]][zref[0] - 16, 0:16, :] = last[0]
                else:
                    rb_[m2[1]][zref[0] - 16, 0:16, :] = last[0].astype(BF16)
                inv_chunk(m2[0], m2[1], i)
        elif m2 is not None and EF:
            for i in range(4):
                inv_chunk(m2[0], m2[1], i)
        if not edep:
            for c in range(LEAD):
                prep(c)
        for j in range(4):
            if not edep:
                for e in range(4):
                    prep(4 * j + e + LEAD)
            if m1 is not None and GP and j < 3:
                zs = pl.ds(pl.multiple_of(zref[0] * 64, 8), 8)
                if 'B' in part:
                    kv32[zs, :] = last[0][0:8]
                if 'C' in part:
                    kt32[zs, :] = lastk[0]
            if m1 is not None:
                for which in ('BC' if BC else 'CB'):
                    if which == 'C' and 'C' in part:
                        fwd_chunk(kt32, sp[m1[1]], 16, j, par[m1[0], 4] if j == 0 else None)
                    if which == 'B' and 'B' in part:
                        fwd_chunk(kv32, sp[m1[1]], 0, j)
            if m2 is not None and not EF and not edep:
                inv_chunk(m2[0], m2[1], j)
            for q in range(4 * j, 4 * j + 4):
                if d is not None:
                    spec_row(d[0], d[1], q)
                if do_gate:
                    gate_block(q)
                if out_g is not None and (q >= 4 or not lag):
                    c = q - 4 if lag else q
                    out_block(out_g, c)
                    if c % 4 == 3:
                        o_copy(out_g, c // 4).start()
        if out_g is not None:
            if lag:
                for c in range(12, 16):
                    out_block(out_g, c)
                o_copy(out_g, 3).start()

    def start(g, m):
        for c in in_copies(g, m):
            c.start()

    def wait(g, m):
        for c in in_copies(g, m):
            c.wait()

    def between(name, fn):
        if NOWHEN:
            fn()
            return
        with jax.named_scope("W_" + name):
            @pl.when(zref[0] > 0)
            def _():
                fn()

    pltpu.make_async_copy(f1_hbm, f1_ref, sem_t.at[0]).start()
    start(0, 0)
    k32[0:8, :] = jnp.zeros((8, 128), F32)
    zref[0] = 32
    for m in range(2):
        shw = sh[m][...].astype(F32)
        dv = dd[m][...].astype(F32)[None, :]
        for g in range(NG):
            for t in range(4):
                par[g * 2 + m, t] = jnp.broadcast_to(shw[t:t + 1, g * 128:(g + 1) * 128], (8, 128))
            par[g * 2 + m, 4] = jnp.broadcast_to(dv[:, g * 128:(g + 1) * 128], (8, 128))

    def wstart(name, before=(), waits=(), after=()):
        def cps(x):
            if x[0] == 'i':
                return in_copies(x[1] // 2, x[1] % 2)
            if x[0] == 'f':
                return in_copies(x[1] // 2, x[1] % 2, 'f')
            if x[0] == 'u':
                return in_copies(x[1] // 2, x[1] % 2, 'kv')
            if x[0] == 't':
                return (pltpu.make_async_copy((f1_hbm, g1_hbm)[x[1]], (f1_ref, g1_ref)[x[1]], sem_t.at[x[1]]),)
            return (q_copy(x[1]),)

        def fn():
            for x in before:
                for c in cps(x):
                    c.start()
            for x in waits:
                for c in cps(x):
                    c.wait()
            for x in after:
                for c in cps(x):
                    c.start()
        between(name, fn)

    wstart("0", waits=[('f', 0), ('t', 0)], after=[('i', 1)])
    if not EXP:
        slot(m1=(0, 0), part='C', tag='0a')
    wstart("0b", waits=[('u', 0)], after=[('i', 2), ('t', 1)])
    if not EXP:
        slot(m1=(0, 0), part='B', tag='0b')
    QS = {1: [0], 2: [1], 3: [2], 4: [3, 4]}
    FS = {7: 0, 8: 1, 9: 2, 10: 3}
    for t in (range(1, 10) if not EXP else EXP):
        before, after = [], []
        if t + 2 <= 9:
            after = [('i', t + 2)]
        after += [('q', g) for g in QS.get(t, [])]
        waits = [('i', t)] + ([('t', 1)] if t == 2 else []) + ([('q', g) for g in range(NG)] if t == 6 else [])
        if SPLIT or t in SPL:
            slot(d=(t - 1, (t - 1) % 2), tag='%d' % t)
            wstart("%d" % t, before, waits, after)
            slot(m1=(t, t % 2), m2=(t - 2, t % 2) if t >= 2 else None,
                 out_g=FS.get(t), do_gate=(t == 6), tag='%d' % t)
        else:
            wstart("%d" % t, before, waits, after)
            slot(d=(t - 1, (t - 1) % 2), m1=(t, t % 2), m2=(t - 2, t % 2) if t >= 2 else None,
                 out_g=FS.get(t), do_gate=(t == 6), tag='%d' % t)
    if not EXP:
        slot(d=(9, 1), m2=(8, 0), out_g=FS.get(10), tag='10')
    slot(m2=(9, 1), out_g=NG - 1, tag='11')
    with jax.named_scope("W_out"):
        for g in range(NG):
            for i in range(4):
                o_copy(g, i).wait()


@jax.jit
def pallas_gated_mix__ssm_conv_h3__ssm_conv_h3__prompt_kernel(
        A_q, A_k, A_v, A_shift_k, A_ssm_k, A_ssm_D,
        B_q, B_k, B_v, B_shift_k, B_ssm_k, B_ssm_D, gate_w):
    hbm = pl.BlockSpec(memory_space=pl.ANY)
    vm = pl.BlockSpec(memory_space=pltpu.VMEM)
    sq = lambda x: x.reshape(S, D)
    out = pl.pallas_call(
        _kernel,
        out_shape=jax.ShapeDtypeStruct((S, D), BF16),
        in_specs=[hbm] * 7 + [vm] * 5 + [hbm] * 2,
        out_specs=hbm,
        scratch_shapes=[
            pltpu.VMEM((4, 128, 128), jnp.uint32),
            pltpu.VMEM((4, 2, 64, 128), jnp.uint32),
            pltpu.SemaphoreType.DMA((2,)),
            pltpu.VMEM((NG, S, 128), BF16),
            pltpu.VMEM((2 * NG, S, 128), BF16),
            pltpu.VMEM((2 * NG, S, 128), BF16),
            pltpu.VMEM((2 * NG, 128, S), BF16),
            pltpu.VMEM((NG, S, 128), BF16),
            pltpu.VMEM((S + 8, 128), F32),
            pltpu.VMEM((S + 8, 128), F32),
            pltpu.VMEM((S + 8, 128), F32),
            pltpu.VMEM((32, 256, 128), F32),
            pltpu.VMEM((32, 256, 128), F32),
            pltpu.VMEM((17, 256, 128), F32),
            pltpu.VMEM((17, 256, 128), F32),
            *[pltpu.VMEM((S, 128), F32) for _ in range(2 * NG)],
            pltpu.VMEM((S, 128), F32),
            pltpu.VMEM((2 * NG, 5, 8, 128), F32),
            pltpu.SemaphoreType.DMA((2 * NG, 3)),
            pltpu.SemaphoreType.DMA((NG,)),
            pltpu.SemaphoreType.DMA((NG, 4)),
            pltpu.SMEM((1,), jnp.int32),
            pltpu.VMEM((17, 256, 128), BF16),
            pltpu.VMEM((17, 256, 128), BF16),
        ],
        compiler_params=pltpu.CompilerParams(vmem_limit_bytes=100 * 1024 * 1024, flags=FLAGS),
    )(sq(A_q), sq(A_k), sq(A_v), A_ssm_k, sq(B_k), sq(B_v), B_ssm_k,
      A_shift_k.T, A_ssm_D, B_shift_k.T, B_ssm_D, gate_w, _F1, _G1)
    return out.reshape(1, S, D)
```

```python
import numpy as np
import jax
import jax.numpy as jnp
import jax.experimental.pallas as pl
import jax.experimental.pallas.tpu as pltpu
import ml_dtypes

S = 2048
D = 640
NG = 5
NI = 2 * NG
M = 1024
F32 = jnp.float32
BF16 = jnp.bfloat16


def _pack_rows(x):
    b = np.ascontiguousarray(x).astype(ml_dtypes.bfloat16).view(np.uint16).astype(np.uint32)
    return b[..., 0::2, :] | (b[..., 1::2, :] << 16)


def _tables():
    k1 = np.concatenate([np.arange(0, 128, 2), np.arange(1, 128, 2)])
    n1 = np.arange(128)
    f = []
    for n2 in range(4):
        e = np.exp(-2j * np.pi * np.outer(k1 + 0.5, 4 * n1 + n2) / M)
        f.append(np.concatenate([e.real, e.imag], 0))
    f = np.stack(f)
    f = f.reshape(4, 2, 16, 8, 128).transpose(0, 2, 1, 3, 4).reshape(4, 256, 128)
    g = np.transpose(f, (0, 2, 1)) * (2.0 / M)
    g = g.reshape(4, 128, 2, 128).transpose(0, 2, 1, 3)
    return _pack_rows(f), _pack_rows(g)


_F1, _G1 = _tables()


def _dft4(x, sign):
    (r0, i0), (r1, i1), (r2, i2), (r3, i3) = x
    ar, ai = r0 + r2, i0 + i2
    br, bi = r0 - r2, i0 - i2
    cr, ci = r1 + r3, i1 + i3
    dr, di = r1 - r3, i1 - i3
    o0 = (ar + cr, ai + ci)
    o2 = (ar - cr, ai - ci)
    op = (br - di, bi + dr)
    om = (br + di, bi - dr)
    return [o0, op, o2, om] if sign > 0 else [o0, om, o2, op]


def _kernel(q_hbm, ak_hbm, av_hbm, af_hbm, bk_hbm, bv_hbm, bf_hbm,
            ash_ref, ad_ref, bsh_ref, bd_ref, gw_ref, f1_hbm, g1_hbm,
            o_hbm,
            f1_ref, g1_ref, q_buf, k_buf, v_buf, f_buf, o_buf,
            k32, kv32, kt32, sp0, sp1, rb0, rb1,
            ya0, ya1, ya2, ya3, ya4, yb0, yb1, yb2, yb3, yb4, gate, par, zref,
            sem_t, sem_in, sem_q, sem_out):
    k_h, v_h, f_h = (ak_hbm, bk_hbm), (av_hbm, bv_hbm), (af_hbm, bf_hbm)
    sp, rb = (sp0, sp1), (rb0, rb1)
    yy = ((ya0, ya1, ya2, ya3, ya4), (yb0, yb1, yb2, yb3, yb4))

    def copies(x):
        kind, n = x
        if kind == 't':
            return [pltpu.make_async_copy((f1_hbm, g1_hbm)[n], (f1_ref, g1_ref)[n], sem_t.at[n])]
        if kind == 'q':
            return [pltpu.make_async_copy(q_hbm.at[:, pl.ds(n * 128, 128)], q_buf.at[n], sem_q.at[n])]
        g, m = divmod(n, 2)
        cols = pl.ds(g * 128, 128)
        out = []
        if kind in 'if':
            out.append(pltpu.make_async_copy(f_h[m].at[cols, :], f_buf.at[n], sem_in.at[n, 0]))
        if kind in 'iu':
            out.append(pltpu.make_async_copy(k_h[m].at[:, cols], k_buf.at[n], sem_in.at[n, 1]))
            out.append(pltpu.make_async_copy(v_h[m].at[:, cols], v_buf.at[n], sem_in.at[n, 2]))
        return out

    def o_copy(g, i):
        rows = pl.ds(512 * i, 512)
        return pltpu.make_async_copy(o_buf.at[g, rows, :], o_hbm.at[rows, pl.ds(g * 128, 128)],
                                     sem_out.at[g, i])

    def dma(name, waits=(), starts=()):
        with jax.named_scope("dma_" + name):
            @pl.when(zref[0] > 0)
            def _():
                for x in waits:
                    for c in copies(x):
                        c.wait()
                for x in starts:
                    for c in copies(x):
                        c.start()

    def tr_block(it, c):
        kt32[c * 128:(c + 1) * 128, :] = f_buf[it, :, c * 128:(c + 1) * 128].astype(F32).T

    def conv_block(it, c):
        rows = pl.ds(128 * c, 128)
        k32[pl.ds(8 + 128 * c, 128), :] = k_buf[it, rows, :].astype(F32)
        acc = None
        for t in range(4):
            x = k32[pl.ds(8 + 128 * c - t, 128), :]
            w = jnp.broadcast_to(par[it, t][0:1, :], (128, 128))
            acc = x * w if acc is None else acc + x * w
        kv = acc * v_buf[it, rows, :].astype(F32)
        kv32[rows, :] = kv
        return kv

    def fwd_chunk(src, dst, off, j, dc=None):
        outs = []
        for n2 in range(4):
            w = src[pl.ds(512 * j + n2, 128, stride=4), :].astype(BF16)
            outs.append(jnp.dot(pltpu.bitcast(f1_ref[n2], BF16), w, preferred_element_type=F32))
        for r in range(16):
            x = _dft4([(o[16 * r:16 * r + 8], o[16 * r + 8:16 * r + 16]) for o in outs], -1)
            for k2 in range(4):
                dst[off + 4 * j + k2, pl.ds(16 * r, 8), :] = x[k2][0] if dc is None else x[k2][0] + dc
                dst[off + 4 * j + k2, pl.ds(16 * r + 8, 8), :] = x[k2][1]

    def spec_row(m, r):
        re, im = pl.ds(16 * r, 8), pl.ds(16 * r + 8, 8)
        s_ = sp[m]
        Y = [[None] * 4 for _ in range(4)]
        for k2 in range(4):
            uu = [(s_[4 * j + k2, re, :], s_[4 * j + k2, im, :]) for j in range(4)]
            kk = [(s_[16 + 4 * j + k2, re, :], s_[16 + 4 * j + k2, im, :]) for j in range(4)]
            kp = [kk[0]]
            for n in range(1, 4):
                pr, pi = kk[n - 1]
                kp.append((kk[n][0] + pi, kk[n][1] - pr) if r >= 8 else (kk[n][0] - pi, kk[n][1] + pr))
            for i in range(4):
                yr = yi = None
                for j in range(i + 1):
                    (ur, ui), (kr, ki) = uu[j], kp[i - j]
                    pr = ur * kr - ui * ki
                    pi = ur * ki + ui * kr
                    yr = pr if yr is None else yr + pr
                    yi = pi if yi is None else yi + pi
                Y[i][k2] = (yr, yi)
        for i in range(4):
            ro = _dft4(Y[i], +1)
            for n2 in range(4):
                rb[m][4 * i + n2, pl.ds(16 * r, 16), :] = jnp.concatenate(ro[n2], axis=0).astype(BF16)

    def inv_chunk(it, i):
        g, m = divmod(it, 2)
        for n2 in range(4):
            p = 4 * i + n2
            y = (jnp.dot(pltpu.bitcast(g1_ref[n2, 0], BF16), rb[m][p, 0:128, :], preferred_element_type=F32)
                 + jnp.dot(pltpu.bitcast(g1_ref[n2, 1], BF16), rb[m][p, 128:256, :], preferred_element_type=F32))
            yy[m][g][pl.ds(512 * i + n2, 128, stride=4), :] = y

    def out_block(g, c):
        rows = pl.ds(128 * c, 128)
        ya, yb = yy[0][g][rows, :], yy[1][g][rows, :]
        o_buf[g, rows, :] = (q_buf[g, rows, :].astype(F32) * (yb + gate[rows, :] * (ya - yb))).astype(BF16)

    def gate_block(c):
        rows = pl.ds(128 * c, 128)
        gw = gw_ref[...].astype(F32)[None, :]
        acc = None
        for g in range(NG):
            t = q_buf[g, rows, :].astype(F32) * gw[:, g * 128:(g + 1) * 128]
            acc = t if acc is None else acc + t
        z = jnp.sum(acc, axis=1, keepdims=True)
        gate[rows, :] = jnp.broadcast_to(0.5 * jnp.tanh(0.5 * z) + 0.5, (128, 128))

    def slot(name, spec=None, fwd=None, inv=None, out_g=None, do_gate=False, part='CB'):
        def prep(c):
            if fwd is None or c >= 16:
                return None
            if 'C' in part:
                tr_block(fwd, c)
            return conv_block(fwd, c) if 'B' in part else None

        lag = inv is not None and out_g is not None and inv == 2 * out_g + 1
        paced = inv is not None and fwd is not None
        with jax.named_scope(name):
            if paced:
                for i in range(4):
                    for e in range(4):
                        kv = prep(4 * i + e)
                    rb[inv % 2][zref[0] - 16, 0:16, :] = kv[112:128, :].astype(BF16)
                    inv_chunk(inv, i)
            else:
                if inv is not None:
                    for i in range(4):
                        inv_chunk(inv, i)
                for c in range(4):
                    prep(c)
            for j in range(4):
                if not paced:
                    for e in range(4):
                        prep(4 * j + e + 4)
                if fwd is not None:
                    if 'C' in part:
                        fwd_chunk(kt32, sp[fwd % 2], 16, j, par[fwd, 4] if j == 0 else None)
                    if 'B' in part:
                        fwd_chunk(kv32, sp[fwd % 2], 0, j)
                for q in range(4 * j, 4 * j + 4):
                    if spec is not None:
                        spec_row(spec % 2, q)
                    if do_gate:
                        gate_block(q)
                    if out_g is not None and (q >= 4 or not lag):
                        c = q - 4 if lag else q
                        out_block(out_g, c)
                        if c % 4 == 3:
                            o_copy(out_g, c // 4).start()
            if lag:
                for c in range(12, 16):
                    out_block(out_g, c)
                o_copy(out_g, 3).start()

    for x in (('t', 0), ('i', 0)):
        for c in copies(x):
            c.start()
    k32[0:8, :] = jnp.zeros((8, 128), F32)
    zref[0] = 32
    for m, (sh_ref, d_ref) in enumerate(((ash_ref, ad_ref), (bsh_ref, bd_ref))):
        shw = sh_ref[...].astype(F32)
        dv = d_ref[...].astype(F32)[None, :]
        for g in range(NG):
            cols = slice(g * 128, (g + 1) * 128)
            for t in range(4):
                par[2 * g + m, t] = jnp.broadcast_to(shw[t:t + 1, cols], (8, 128))
            par[2 * g + m, 4] = jnp.broadcast_to(dv[:, cols], (8, 128))

    dma("0a", waits=[('f', 0), ('t', 0)], starts=[('i', 1)])
    slot("step0a", fwd=0, part='C')
    dma("0b", waits=[('u', 0)], starts=[('i', 2), ('t', 1)])
    slot("step0b", fwd=0, part='B')
    q_at = {1: [0], 2: [1], 3: [2], 4: [3, 4]}
    out_at = {7: 0, 8: 1, 9: 2, 10: 3}
    for t in range(1, NI):
        waits = [('i', t)] + ([('t', 1)] if t == 2 else []) + ([('q', g) for g in range(NG)] if t == 6 else [])
        starts = ([('i', t + 2)] if t + 2 < NI else []) + [('q', g) for g in q_at.get(t, [])]
        if t == 1:
            slot("step1a", spec=0)
            dma("1", waits, starts)
            slot("step1b", fwd=1)
        else:
            dma("%d" % t, waits, starts)
            slot("step%d" % t, spec=t - 1, fwd=t, inv=t - 2, out_g=out_at.get(t), do_gate=(t == 6))
    slot("step10", spec=NI - 1, inv=NI - 2, out_g=out_at[10])
    slot("step11", inv=NI - 1, out_g=NG - 1)
    with jax.named_scope("dma_out"):
        for g in range(NG):
            for i in range(4):
                o_copy(g, i).wait()


@jax.jit
def pallas_gated_mix__ssm_conv_h3__ssm_conv_h3__prompt_kernel(
        A_q, A_k, A_v, A_shift_k, A_ssm_k, A_ssm_D,
        B_q, B_k, B_v, B_shift_k, B_ssm_k, B_ssm_D, gate_w):
    del B_q
    hbm = pl.BlockSpec(memory_space=pl.ANY)
    vmem = pl.BlockSpec(memory_space=pltpu.VMEM)
    sq = lambda x: x.reshape(S, D)
    out = pl.pallas_call(
        _kernel,
        out_shape=jax.ShapeDtypeStruct((S, D), BF16),
        in_specs=[hbm] * 7 + [vmem] * 5 + [hbm] * 2,
        out_specs=hbm,
        scratch_shapes=[
            pltpu.VMEM((4, 128, 128), jnp.uint32),
            pltpu.VMEM((4, 2, 64, 128), jnp.uint32),
            pltpu.VMEM((NG, S, 128), BF16),
            pltpu.VMEM((NI, S, 128), BF16),
            pltpu.VMEM((NI, S, 128), BF16),
            pltpu.VMEM((NI, 128, S), BF16),
            pltpu.VMEM((NG, S, 128), BF16),
            pltpu.VMEM((S + 8, 128), F32),
            pltpu.VMEM((S, 128), F32),
            pltpu.VMEM((S, 128), F32),
            pltpu.VMEM((32, 256, 128), F32),
            pltpu.VMEM((32, 256, 128), F32),
            pltpu.VMEM((17, 256, 128), BF16),
            pltpu.VMEM((17, 256, 128), BF16),
            *[pltpu.VMEM((S, 128), F32) for _ in range(NI)],
            pltpu.VMEM((S, 128), F32),
            pltpu.VMEM((NI, 5, 8, 128), F32),
            pltpu.SMEM((1,), jnp.int32),
            pltpu.SemaphoreType.DMA((2,)),
            pltpu.SemaphoreType.DMA((NI, 3)),
            pltpu.SemaphoreType.DMA((NG,)),
            pltpu.SemaphoreType.DMA((NG, 4)),
        ],
        compiler_params=pltpu.CompilerParams(
            vmem_limit_bytes=100 * 1024 * 1024,
            flags={"XLA_TPU_EVENLY_DISTRIBUTE_CRITICAL_NODES": True}),
    )(sq(A_q), sq(A_k), sq(A_v), A_ssm_k, sq(B_k), sq(B_v), B_ssm_k,
      A_shift_k.T, A_ssm_D, B_shift_k.T, B_ssm_D, gate_w, _F1, _G1)
    return out.reshape(1, S, D)
```

```python
import numpy as np
import jax
import jax.numpy as jnp
import jax.experimental.pallas as pl
import jax.experimental.pallas.tpu as pltpu
import ml_dtypes

S = 2048
D = 640
NG = 5
NI = 2 * NG
M = 1024
F32 = jnp.float32
BF16 = jnp.bfloat16


def _pack_rows(x):
    b = np.ascontiguousarray(x).astype(ml_dtypes.bfloat16).view(np.uint16).astype(np.uint32)
    return b[..., 0::2, :] | (b[..., 1::2, :] << 16)


def _tables():
    k1 = np.concatenate([np.arange(0, 128, 2), np.arange(1, 128, 2)])
    n1 = np.arange(128)
    f = []
    for n2 in range(4):
        e = np.exp(-2j * np.pi * np.outer(k1 + 0.5, 4 * n1 + n2) / M)
        f.append(np.concatenate([e.real, e.imag], 0))
    f = np.stack(f)
    f = f.reshape(4, 2, 16, 8, 128).transpose(0, 2, 1, 3, 4).reshape(4, 256, 128)
    g = np.transpose(f, (0, 2, 1)) * (2.0 / M)
    g = g.reshape(4, 128, 2, 128).transpose(0, 2, 1, 3)
    return _pack_rows(f), _pack_rows(g)


_F1, _G1 = _tables()


def _dft4(x, sign):
    (r0, i0), (r1, i1), (r2, i2), (r3, i3) = x
    ar, ai = r0 + r2, i0 + i2
    br, bi = r0 - r2, i0 - i2
    cr, ci = r1 + r3, i1 + i3
    dr, di = r1 - r3, i1 - i3
    o0 = (ar + cr, ai + ci)
    o2 = (ar - cr, ai - ci)
    op = (br - di, bi + dr)
    om = (br + di, bi - dr)
    return [o0, op, o2, om] if sign > 0 else [o0, om, o2, op]


def _kernel(q_hbm, ak_hbm, av_hbm, af_hbm, bk_hbm, bv_hbm, bf_hbm,
            ash_ref, ad_ref, bsh_ref, bd_ref, gw_ref, f1_hbm, g1_hbm,
            o_hbm,
            f1_ref, g1_ref, q_buf, k_buf, v_buf, f_buf, o_buf,
            k32, kv32, kt32, sp0, sp1, rb0, rb1,
            ya0, ya1, ya2, ya3, ya4, yb0, yb1, yb2, yb3, yb4, gate, par, zref,
            sem_t, sem_in, sem_q, sem_out):
    k_h, v_h, f_h = (ak_hbm, bk_hbm), (av_hbm, bv_hbm), (af_hbm, bf_hbm)
    sp, rb = (sp0, sp1), (rb0, rb1)
    yy = ((ya0, ya1, ya2, ya3, ya4), (yb0, yb1, yb2, yb3, yb4))

    def copies(x):
        kind, n = x
        if kind == 't':
            return [pltpu.make_async_copy((f1_hbm, g1_hbm)[n], (f1_ref, g1_ref)[n], sem_t.at[n])]
        if kind == 'q':
            return [pltpu.make_async_copy(q_hbm.at[:, pl.ds(n * 128, 128)], q_buf.at[n], sem_q.at[n])]
        g, m = divmod(n, 2)
        cols = pl.ds(g * 128, 128)
        out = []
        if kind in 'if':
            out.append(pltpu.make_async_copy(f_h[m].at[cols, :], f_buf.at[n], sem_in.at[n, 0]))
        if kind in 'iu':
            out.append(pltpu.make_async_copy(k_h[m].at[:, cols], k_buf.at[n], sem_in.at[n, 1]))
            out.append(pltpu.make_async_copy(v_h[m].at[:, cols], v_buf.at[n], sem_in.at[n, 2]))
        return out

    def o_copy(g, i):
        rows = pl.ds(512 * i, 512)
        return pltpu.make_async_copy(o_buf.at[g, rows, :], o_hbm.at[rows, pl.ds(g * 128, 128)],
                                     sem_out.at[g, i])

    def dma(name, waits=(), starts=()):
        with jax.named_scope("dma_" + name):
            @pl.when(zref[0] > 0)
            def _():
                for x in waits:
                    for c in copies(x):
                        c.wait()
                for x in starts:
                    for c in copies(x):
                        c.start()

    def tr_block(it, c):
        kt32[c * 128:(c + 1) * 128, :] = f_buf[it, :, c * 128:(c + 1) * 128].astype(F32).T

    def conv_block(it, c):
        rows = pl.ds(128 * c, 128)
        k32[pl.ds(8 + 128 * c, 128), :] = k_buf[it, rows, :].astype(F32)
        acc = None
        for t in range(4):
            x = k32[pl.ds(8 + 128 * c - t, 128), :]
            w = jnp.broadcast_to(par[it, t][0:1, :], (128, 128))
            acc = x * w if acc is None else acc + x * w
        kv = acc * v_buf[it, rows, :].astype(F32)
        kv32[rows, :] = kv
        return kv

    def fwd_chunk(src, dst, off, j, dc=None):
        outs = []
        for n2 in range(4):
            w = src[pl.ds(512 * j + n2, 128, stride=4), :].astype(BF16)
            outs.append(jnp.dot(pltpu.bitcast(f1_ref[n2], BF16), w, preferred_element_type=F32))
        for r in range(16):
            x = _dft4([(o[16 * r:16 * r + 8], o[16 * r + 8:16 * r + 16]) for o in outs], -1)
            for k2 in range(4):
                dst[off + 4 * j + k2, pl.ds(16 * r, 8), :] = x[k2][0] if dc is None else x[k2][0] + dc
                dst[off + 4 * j + k2, pl.ds(16 * r + 8, 8), :] = x[k2][1]

    def spec_row(m, r):
        re, im = pl.ds(16 * r, 8), pl.ds(16 * r + 8, 8)
        s_ = sp[m]
        Y = [[None] * 4 for _ in range(4)]
        for k2 in range(4):
            uu = [(s_[4 * j + k2, re, :], s_[4 * j + k2, im, :]) for j in range(4)]
            kk = [(s_[16 + 4 * j + k2, re, :], s_[16 + 4 * j + k2, im, :]) for j in range(4)]
            kp = [kk[0]]
            for n in range(1, 4):
                pr, pi = kk[n - 1]
                kp.append((kk[n][0] + pi, kk[n][1] - pr) if r >= 8 else (kk[n][0] - pi, kk[n][1] + pr))
            k3 = [(kr, ki - kr, kr + ki) for kr, ki in kp]
            u3 = [(ur + ui, ur, ui) for ur, ui in uu]
            for i in range(4):
                a = b = c = None
                for j in range(i + 1):
                    (us, ur, ui), (kr, km, kq) = u3[j], k3[i - j]
                    a = kr * us if a is None else a + kr * us
                    b = ur * km if b is None else b + ur * km
                    c = ui * kq if c is None else c + ui * kq
                Y[i][k2] = (a - c, a + b)
        for i in range(4):
            ro = _dft4(Y[i], +1)
            for n2 in range(4):
                rb[m][4 * i + n2, pl.ds(16 * r, 16), :] = jnp.concatenate(ro[n2], axis=0).astype(BF16)

    def inv_chunk(it, i):
        g, m = divmod(it, 2)
        for n2 in range(4):
            p = 4 * i + n2
            y = (jnp.dot(pltpu.bitcast(g1_ref[n2, 0], BF16), rb[m][p, 0:128, :], preferred_element_type=F32)
                 + jnp.dot(pltpu.bitcast(g1_ref[n2, 1], BF16), rb[m][p, 128:256, :], preferred_element_type=F32))
            yy[m][g][pl.ds(512 * i + n2, 128, stride=4), :] = y

    def out_block(g, c):
        rows = pl.ds(128 * c, 128)
        ya, yb = yy[0][g][rows, :], yy[1][g][rows, :]
        o_buf[g, rows, :] = (q_buf[g, rows, :].astype(F32) * (yb + gate[rows, :] * (ya - yb))).astype(BF16)

    def gate_block(c):
        rows = pl.ds(128 * c, 128)
        gw = gw_ref[...].astype(F32)[None, :]
        acc = None
        for g in range(NG):
            t = q_buf[g, rows, :].astype(F32) * gw[:, g * 128:(g + 1) * 128]
            acc = t if acc is None else acc + t
        z = jnp.sum(acc, axis=1, keepdims=True)
        gate[rows, :] = jnp.broadcast_to(0.5 * jnp.tanh(0.5 * z) + 0.5, (128, 128))

    def slot(name, spec=None, fwd=None, inv=None, out_g=None, do_gate=False, part='CB'):
        def prep(c):
            if fwd is None or c >= 16:
                return None
            if 'C' in part:
                tr_block(fwd, c)
            return conv_block(fwd, c) if 'B' in part else None

        lag = inv is not None and out_g is not None and inv == 2 * out_g + 1
        paced = inv is not None and fwd is not None and out_g is None and not do_gate
        with jax.named_scope(name):
            if paced:
                for i in range(4):
                    for e in range(4):
                        kv = prep(4 * i + e)
                    rb[inv % 2][zref[0] - 16, 0:16, :] = kv[112:128, :].astype(BF16)
                    inv_chunk(inv, i)
            else:
                if inv is not None:
                    for i in range(4):
                        inv_chunk(inv, i)
                for c in range(4):
                    prep(c)
            for j in range(4):
                if not paced:
                    for e in range(4):
                        prep(4 * j + e + 4)
                if fwd is not None:
                    if 'C' in part:
                        fwd_chunk(kt32, sp[fwd % 2], 16, j, par[fwd, 4] if j == 0 else None)
                    if 'B' in part:
                        fwd_chunk(kv32, sp[fwd % 2], 0, j)
                for q in range(4 * j, 4 * j + 4):
                    if spec is not None:
                        spec_row(spec % 2, q)
                    if do_gate:
                        gate_block(q)
                    if out_g is not None and (q >= 4 or not lag):
                        c = q - 4 if lag else q
                        out_block(out_g, c)
                        if c % 4 == 3:
                            o_copy(out_g, c // 4).start()
            if lag:
                for c in range(12, 16):
                    out_block(out_g, c)
                o_copy(out_g, 3).start()

    for x in (('t', 0), ('i', 0)):
        for c in copies(x):
            c.start()
    k32[0:8, :] = jnp.zeros((8, 128), F32)
    zref[0] = 32
    for m, (sh_ref, d_ref) in enumerate(((ash_ref, ad_ref), (bsh_ref, bd_ref))):
        shw = sh_ref[...].astype(F32)
        dv = d_ref[...].astype(F32)[None, :]
        for g in range(NG):
            cols = slice(g * 128, (g + 1) * 128)
            for t in range(4):
                par[2 * g + m, t] = jnp.broadcast_to(shw[t:t + 1, cols], (8, 128))
            par[2 * g + m, 4] = jnp.broadcast_to(dv[:, cols], (8, 128))

    dma("0a", waits=[('f', 0), ('t', 0)], starts=[('i', 1)])
    slot("step0a", fwd=0, part='C')
    dma("0b", waits=[('u', 0)], starts=[('i', 2), ('t', 1)])
    slot("step0b", fwd=0, part='B')
    q_at = {1: [0], 2: [1], 3: [2], 4: [3, 4]}
    out_at = {7: 0, 8: 1, 9: 2, 10: 3}
    for t in range(1, NI):
        waits = [('i', t)] + ([('t', 1)] if t == 2 else []) + ([('q', g) for g in range(NG)] if t == 6 else [])
        starts = ([('i', t + 2)] if t + 2 < NI else []) + [('q', g) for g in q_at.get(t, [])]
        if t == 1:
            slot("step1a", spec=0)
            dma("1", waits, starts)
            slot("step1b", fwd=1)
        else:
            dma("%d" % t, waits, starts)
            slot("step%d" % t, spec=t - 1, fwd=t, inv=t - 2, out_g=out_at.get(t), do_gate=(t == 6))
    slot("step10", spec=NI - 1, inv=NI - 2, out_g=out_at[10])
    slot("step11", inv=NI - 1, out_g=NG - 1)
    with jax.named_scope("dma_out"):
        for g in range(NG):
            for i in range(4):
                o_copy(g, i).wait()


@jax.jit
def pallas_gated_mix__ssm_conv_h3__ssm_conv_h3__prompt_kernel(
        A_q, A_k, A_v, A_shift_k, A_ssm_k, A_ssm_D,
        B_q, B_k, B_v, B_shift_k, B_ssm_k, B_ssm_D, gate_w):
    del B_q
    hbm = pl.BlockSpec(memory_space=pl.ANY)
    vmem = pl.BlockSpec(memory_space=pltpu.VMEM)
    sq = lambda x: x.reshape(S, D)
    out = pl.pallas_call(
        _kernel,
        out_shape=jax.ShapeDtypeStruct((S, D), BF16),
        in_specs=[hbm] * 7 + [vmem] * 5 + [hbm] * 2,
        out_specs=hbm,
        scratch_shapes=[
            pltpu.VMEM((4, 128, 128), jnp.uint32),
            pltpu.VMEM((4, 2, 64, 128), jnp.uint32),
            pltpu.VMEM((NG, S, 128), BF16),
            pltpu.VMEM((NI, S, 128), BF16),
            pltpu.VMEM((NI, S, 128), BF16),
            pltpu.VMEM((NI, 128, S), BF16),
            pltpu.VMEM((NG, S, 128), BF16),
            pltpu.VMEM((S + 8, 128), F32),
            pltpu.VMEM((S, 128), F32),
            pltpu.VMEM((S, 128), F32),
            pltpu.VMEM((32, 256, 128), F32),
            pltpu.VMEM((32, 256, 128), F32),
            pltpu.VMEM((17, 256, 128), BF16),
            pltpu.VMEM((17, 256, 128), BF16),
            *[pltpu.VMEM((S, 128), F32) for _ in range(NI)],
            pltpu.VMEM((S, 128), F32),
            pltpu.VMEM((NI, 5, 8, 128), F32),
            pltpu.SMEM((1,), jnp.int32),
            pltpu.SemaphoreType.DMA((2,)),
            pltpu.SemaphoreType.DMA((NI, 3)),
            pltpu.SemaphoreType.DMA((NG,)),
            pltpu.SemaphoreType.DMA((NG, 4)),
        ],
        compiler_params=pltpu.CompilerParams(
            vmem_limit_bytes=100 * 1024 * 1024,
            flags={"XLA_TPU_EVENLY_DISTRIBUTE_CRITICAL_NODES": True}),
    )(sq(A_q), sq(A_k), sq(A_v), A_ssm_k, sq(B_k), sq(B_v), B_ssm_k,
      A_shift_k.T, A_ssm_D, B_shift_k.T, B_ssm_D, gate_w, _F1, _G1)
    return out.reshape(1, S, D)
```

```python
import numpy as np
import jax
import jax.numpy as jnp
import jax.experimental.pallas as pl
import jax.experimental.pallas.tpu as pltpu
import ml_dtypes

S = 2048
D = 640
NG = 5
NI = 2 * NG
M = 1024
F32 = jnp.float32
BF16 = jnp.bfloat16


def _pack_rows(x):
    b = np.ascontiguousarray(x).astype(ml_dtypes.bfloat16).view(np.uint16).astype(np.uint32)
    return b[..., 0::2, :] | (b[..., 1::2, :] << 16)


def _tables():
    k1 = np.concatenate([np.arange(0, 128, 2), np.arange(1, 128, 2)])
    n1 = np.arange(128)
    f = []
    for n2 in range(4):
        e = np.exp(-2j * np.pi * np.outer(k1 + 0.5, 4 * n1 + n2) / M)
        f.append(np.concatenate([e.real, e.imag], 0))
    f = np.stack(f)
    f = f.reshape(4, 2, 16, 8, 128).transpose(0, 2, 1, 3, 4).reshape(4, 256, 128)
    g = np.transpose(f, (0, 2, 1)) * (2.0 / M)
    g = g.reshape(4, 128, 2, 128).transpose(0, 2, 1, 3)
    return _pack_rows(f), _pack_rows(g)


_F1, _G1 = _tables()


def _dft4(x, sign):
    (r0, i0), (r1, i1), (r2, i2), (r3, i3) = x
    ar, ai = r0 + r2, i0 + i2
    br, bi = r0 - r2, i0 - i2
    cr, ci = r1 + r3, i1 + i3
    dr, di = r1 - r3, i1 - i3
    o0 = (ar + cr, ai + ci)
    o2 = (ar - cr, ai - ci)
    op = (br - di, bi + dr)
    om = (br + di, bi - dr)
    return [o0, op, o2, om] if sign > 0 else [o0, om, o2, op]


def _kernel(q_hbm, ak_hbm, av_hbm, af_hbm, bk_hbm, bv_hbm, bf_hbm,
            ash_ref, ad_ref, bsh_ref, bd_ref, gw_ref, f1_hbm, g1_hbm,
            o_hbm,
            f1_ref, g1_ref, q_buf, k_buf, v_buf, f_buf, o_buf,
            k32, kv32, kt32, sp0, sp1, rb0, rb1,
            ya0, ya1, ya2, ya3, ya4, yb0, yb1, yb2, yb3, yb4, gate, par, zref,
            sem_t, sem_in, sem_q, sem_out):
    k_h, v_h, f_h = (ak_hbm, bk_hbm), (av_hbm, bv_hbm), (af_hbm, bf_hbm)
    sp, rb = (sp0, sp1), (rb0, rb1)
    yy = ((ya0, ya1, ya2, ya3, ya4), (yb0, yb1, yb2, yb3, yb4))

    def copies(x):
        kind, n = x
        if kind == 't':
            return [pltpu.make_async_copy((f1_hbm, g1_hbm)[n], (f1_ref, g1_ref)[n], sem_t.at[n])]
        if kind == 'q':
            return [pltpu.make_async_copy(q_hbm.at[:, pl.ds(n * 128, 128)], q_buf.at[n], sem_q.at[n])]
        g, m = divmod(n, 2)
        cols = pl.ds(g * 128, 128)
        out = []
        if kind in 'if':
            out.append(pltpu.make_async_copy(f_h[m].at[cols, :], f_buf.at[n], sem_in.at[n, 0]))
        if kind in 'iu':
            out.append(pltpu.make_async_copy(k_h[m].at[:, cols], k_buf.at[n], sem_in.at[n, 1]))
            out.append(pltpu.make_async_copy(v_h[m].at[:, cols], v_buf.at[n], sem_in.at[n, 2]))
        return out

    def o_copy(g, i):
        rows = pl.ds(512 * i, 512)
        return pltpu.make_async_copy(o_buf.at[g, rows, :], o_hbm.at[rows, pl.ds(g * 128, 128)],
                                     sem_out.at[g, i])

    def dma(name, waits=(), starts=()):
        with jax.named_scope("dma_" + name):
            @pl.when(zref[0] > 0)
            def _():
                for x in waits:
                    for c in copies(x):
                        c.wait()
                for x in starts:
                    for c in copies(x):
                        c.start()

    def tr_block(it, c):
        kt32[c * 128:(c + 1) * 128, :] = f_buf[it, :, c * 128:(c + 1) * 128].astype(F32).T

    def conv_block(it, c):
        rows = pl.ds(128 * c, 128)
        k32[pl.ds(8 + 128 * c, 128), :] = k_buf[it, rows, :].astype(F32)
        acc = None
        for t in range(4):
            x = k32[pl.ds(8 + 128 * c - t, 128), :]
            w = jnp.broadcast_to(par[it, t][0:1, :], (128, 128))
            acc = x * w if acc is None else acc + x * w
        kv = acc * v_buf[it, rows, :].astype(F32)
        kv32[rows, :] = kv
        return kv

    def fwd_chunk(src, dst, off, j, dc=None):
        outs = []
        for n2 in range(4):
            w = src[pl.ds(512 * j + n2, 128, stride=4), :].astype(BF16)
            outs.append(jnp.dot(pltpu.bitcast(f1_ref[n2], BF16), w, preferred_element_type=F32))
        for r in range(16):
            x = _dft4([(o[16 * r:16 * r + 8], o[16 * r + 8:16 * r + 16]) for o in outs], -1)
            for k2 in range(4):
                dst[off + 4 * j + k2, pl.ds(16 * r, 8), :] = x[k2][0] if dc is None else x[k2][0] + dc
                dst[off + 4 * j + k2, pl.ds(16 * r + 8, 8), :] = x[k2][1]

    def spec_row(m, r):
        re, im = pl.ds(16 * r, 8), pl.ds(16 * r + 8, 8)
        s_ = sp[m]
        Y = [[None] * 4 for _ in range(4)]
        for k2 in range(4):
            uu = [(s_[4 * j + k2, re, :], s_[4 * j + k2, im, :]) for j in range(4)]
            kk = [(s_[16 + 4 * j + k2, re, :], s_[16 + 4 * j + k2, im, :]) for j in range(4)]
            kp = [kk[0]]
            for n in range(1, 4):
                pr, pi = kk[n - 1]
                kp.append((kk[n][0] + pi, kk[n][1] - pr) if r >= 8 else (kk[n][0] - pi, kk[n][1] + pr))
            k3 = [(kr, ki - kr, kr + ki) for kr, ki in kp]
            u3 = [(ur + ui, ur, ui) for ur, ui in uu]
            for i in range(4):
                a = b = c = None
                for j in range(i + 1):
                    (us, ur, ui), (kr, km, kq) = u3[j], k3[i - j]
                    a = kr * us if a is None else a + kr * us
                    b = ur * km if b is None else b + ur * km
                    c = ui * kq if c is None else c + ui * kq
                Y[i][k2] = (a - c, a + b)
        for i in range(4):
            ro = _dft4(Y[i], +1)
            for n2 in range(4):
                rb[m][4 * i + n2, pl.ds(16 * r, 16), :] = jnp.concatenate(ro[n2], axis=0).astype(BF16)

    def inv_chunk(it, i):
        g, m = divmod(it, 2)
        for n2 in range(4):
            p = 4 * i + n2
            y = (jnp.dot(pltpu.bitcast(g1_ref[n2, 0], BF16), rb[m][p, 0:128, :], preferred_element_type=F32)
                 + jnp.dot(pltpu.bitcast(g1_ref[n2, 1], BF16), rb[m][p, 128:256, :], preferred_element_type=F32))
            yy[m][g][pl.ds(512 * i + n2, 128, stride=4), :] = y

    def out_block(g, c):
        rows = pl.ds(128 * c, 128)
        ya, yb = yy[0][g][rows, :], yy[1][g][rows, :]
        o_buf[g, rows, :] = (q_buf[g, rows, :].astype(F32) * (yb + gate[rows, :] * (ya - yb))).astype(BF16)

    def gate_block(c):
        rows = pl.ds(128 * c, 128)
        gw = gw_ref[...].astype(F32)[None, :]
        acc = None
        for g in range(NG):
            t = q_buf[g, rows, :].astype(F32) * gw[:, g * 128:(g + 1) * 128]
            acc = t if acc is None else acc + t
        z = jnp.sum(acc, axis=1, keepdims=True)
        gate[rows, :] = jnp.broadcast_to(0.5 * jnp.tanh(0.5 * z) + 0.5, (128, 128))

    def slot(name, spec=None, fwd=None, inv=None, out_g=None, do_gate=False, part='CB'):
        def prep(c):
            if fwd is None or c >= 16:
                return None
            if 'C' in part:
                tr_block(fwd, c)
            return conv_block(fwd, c) if 'B' in part else None

        lag = inv is not None and out_g is not None and inv == 2 * out_g + 1
        paced = inv is not None and fwd is not None
        with jax.named_scope(name):
            if paced:
                for i in range(4):
                    for e in range(3):
                        kv = prep(4 * i + e)
                    rb[inv % 2][zref[0] - 16, 0:16, :] = kv[112:128, :].astype(BF16)
                    inv_chunk(inv, i)
                    for e in range(3, 4):
                        prep(4 * i + e)
            else:
                if inv is not None:
                    for i in range(4):
                        inv_chunk(inv, i)
                for c in range(4):
                    prep(c)
            for j in range(4):
                if not paced:
                    for e in range(4):
                        prep(4 * j + e + 4)
                if fwd is not None:
                    if 'C' in part:
                        fwd_chunk(kt32, sp[fwd % 2], 16, j, par[fwd, 4] if j == 0 else None)
                    if 'B' in part:
                        fwd_chunk(kv32, sp[fwd % 2], 0, j)
                for q in range(4 * j, 4 * j + 4):
                    if spec is not None:
                        spec_row(spec % 2, q)
                    if do_gate:
                        gate_block(q)
                    if out_g is not None and (q >= 4 or not lag):
                        c = q - 4 if lag else q
                        out_block(out_g, c)
                        if c % 4 == 3:
                            o_copy(out_g, c // 4).start()
            if lag:
                for c in range(12, 16):
                    out_block(out_g, c)
                o_copy(out_g, 3).start()

    for x in (('t', 0), ('i', 0)):
        for c in copies(x):
            c.start()
    k32[0:8, :] = jnp.zeros((8, 128), F32)
    zref[0] = 32
    for m, (sh_ref, d_ref) in enumerate(((ash_ref, ad_ref), (bsh_ref, bd_ref))):
        shw = sh_ref[...].astype(F32)
        dv = d_ref[...].astype(F32)[None, :]
        for g in range(NG):
            cols = slice(g * 128, (g + 1) * 128)
            for t in range(4):
                par[2 * g + m, t] = jnp.broadcast_to(shw[t:t + 1, cols], (8, 128))
            par[2 * g + m, 4] = jnp.broadcast_to(dv[:, cols], (8, 128))

    dma("0a", waits=[('f', 0), ('t', 0)], starts=[('i', 1)])
    slot("step0a", fwd=0, part='C')
    dma("0b", waits=[('u', 0)], starts=[('i', 2), ('t', 1)])
    slot("step0b", fwd=0, part='B')
    q_at = {1: [0], 2: [1], 3: [2], 4: [3, 4]}
    out_at = {7: 0, 8: 1, 9: 2, 10: 3}
    for t in range(1, NI):
        waits = [('i', t)] + ([('t', 1)] if t == 2 else []) + ([('q', g) for g in range(NG)] if t == 6 else [])
        starts = ([('i', t + 2)] if t + 2 < NI else []) + [('q', g) for g in q_at.get(t, [])]
        if t == 1:
            slot("step1a", spec=0)
            dma("1", waits, starts)
            slot("step1b", fwd=1)
        else:
            dma("%d" % t, waits, starts)
            slot("step%d" % t, spec=t - 1, fwd=t, inv=t - 2, out_g=out_at.get(t), do_gate=(t == 6))
    slot("step10", spec=NI - 1, inv=NI - 2, out_g=out_at[10])
    slot("step11", inv=NI - 1, out_g=NG - 1)
    with jax.named_scope("dma_out"):
        for g in range(NG):
            for i in range(4):
                o_copy(g, i).wait()


@jax.jit
def pallas_gated_mix__ssm_conv_h3__ssm_conv_h3__prompt_kernel(
        A_q, A_k, A_v, A_shift_k, A_ssm_k, A_ssm_D,
        B_q, B_k, B_v, B_shift_k, B_ssm_k, B_ssm_D, gate_w):
    del B_q
    hbm = pl.BlockSpec(memory_space=pl.ANY)
    vmem = pl.BlockSpec(memory_space=pltpu.VMEM)
    sq = lambda x: x.reshape(S, D)
    out = pl.pallas_call(
        _kernel,
        out_shape=jax.ShapeDtypeStruct((S, D), BF16),
        in_specs=[hbm] * 7 + [vmem] * 5 + [hbm] * 2,
        out_specs=hbm,
        scratch_shapes=[
            pltpu.VMEM((4, 128, 128), jnp.uint32),
            pltpu.VMEM((4, 2, 64, 128), jnp.uint32),
            pltpu.VMEM((NG, S, 128), BF16),
            pltpu.VMEM((NI, S, 128), BF16),
            pltpu.VMEM((NI, S, 128), BF16),
            pltpu.VMEM((NI, 128, S), BF16),
            pltpu.VMEM((NG, S, 128), BF16),
            pltpu.VMEM((S + 8, 128), F32),
            pltpu.VMEM((S, 128), F32),
            pltpu.VMEM((S, 128), F32),
            pltpu.VMEM((32, 256, 128), F32),
            pltpu.VMEM((32, 256, 128), F32),
            pltpu.VMEM((17, 256, 128), BF16),
            pltpu.VMEM((17, 256, 128), BF16),
            *[pltpu.VMEM((S, 128), F32) for _ in range(NI)],
            pltpu.VMEM((S, 128), F32),
            pltpu.VMEM((NI, 5, 8, 128), F32),
            pltpu.SMEM((1,), jnp.int32),
            pltpu.SemaphoreType.DMA((2,)),
            pltpu.SemaphoreType.DMA((NI, 3)),
            pltpu.SemaphoreType.DMA((NG,)),
            pltpu.SemaphoreType.DMA((NG, 4)),
        ],
        compiler_params=pltpu.CompilerParams(
            vmem_limit_bytes=100 * 1024 * 1024,
            flags={"XLA_TPU_EVENLY_DISTRIBUTE_CRITICAL_NODES": True}),
    )(sq(A_q), sq(A_k), sq(A_v), A_ssm_k, sq(B_k), sq(B_v), B_ssm_k,
      A_shift_k.T, A_ssm_D, B_shift_k.T, B_ssm_D, gate_w, _F1, _G1)
    return out.reshape(1, S, D)
```
